```python
import jax
import jax.numpy as jnp

def _softmax(x, axis=-1):
    return jax.nn.softmax(x, axis=axis)

def _gelu(x):
    return jax.nn.gelu(x, approximate=True)

def _silu(x):
    return jax.nn.silu(x)

def _sigmoid(x):
    return jax.nn.sigmoid(x)

def _layernorm(x, axis=-1, eps=1e-05):
    m = jnp.mean(x, axis=axis, keepdims=True)
    v = jnp.var(x, axis=axis, keepdims=True)
    return (x - m) / jnp.sqrt(v + eps)

def _scatter_add(tgt, idx, src, axis=0):
    return tgt.at[idx].add(src)

def _segment_sum(src, seg, n):
    return jax.ops.segment_sum(src, seg, n)

class _Rng:

    def __init__(self, key):
        self._k = key

    def _next(self):
        self._k, sub = jax.random.split(self._k)
        return sub

    def normal(self, shape):
        return jax.random.normal(self._next(), shape, dtype=jnp.bfloat16)

    def randint(self, lo, hi, shape):
        return jax.random.randint(self._next(), shape, lo, hi, dtype=jnp.int32)

    def uniform(self, shape, lo=0.0, hi=1.0):
        return jax.random.uniform(self._next(), shape, jnp.bfloat16, lo, hi)

    def permutation(self, n):
        return jax.random.permutation(self._next(), n)
kernel_name = 'concat_heads__memory_aug_recurrent_mem_tr__compressed_kv_cla__prompt'

def setup_inputs():
    _rng = _Rng(jax.random.key(int.from_bytes(__import__("os").urandom(4), "little")))
    _w = lambda a: (lambda t: t.astype(jnp.bfloat16) if jnp.issubdtype(t.dtype, jnp.floating) else t)(jnp.asarray(a))

    def _A_setup():
        B, S, Dm = (1, 2048, 448)
        H, Dh = (16, 256)
        M, seg = (8, 32)
        seg = min(seg, S)
        S = S // seg * seg
        return {'x': _w((lambda *s: _rng.normal(s) * 0.05)(B, S, Dm)), 'mem0': _w((lambda *s: _rng.normal(s) * 0.05)(B, M, Dm)), 'Wq': _w((lambda *s: _rng.normal(s) * 0.05)(Dm, H, Dh) * Dm ** (-0.5)), 'Wk': _w((lambda *s: _rng.normal(s) * 0.05)(Dm, H, Dh) * Dm ** (-0.5)), 'Wv': _w((lambda *s: _rng.normal(s) * 0.05)(Dm, H, Dh) * Dm ** (-0.5)), 'Wo': _w((lambda *s: _rng.normal(s) * 0.05)(H, Dh, Dm) * (H * Dh) ** (-0.5)), 'seg_len': seg}
    _A_in = _A_setup()

    def _B_setup():
        B, H, Sq, Sk, D, M = (1, 16, 2048, 2048, 256, 448)
        Dc = 4 * D
        return {'x': _w((lambda *s: _rng.normal(s) * 0.05)(B, Sq, M)), 'c_kv': _w((lambda *s: _rng.normal(s) * 0.05)(B, Sk, Dc)), 'w_q': _w((lambda *s: _rng.normal(s) * 0.05)(M, H, D) * M ** (-0.5)), 'w_uk': _w((lambda *s: _rng.normal(s) * 0.05)(Dc, H, D) * Dc ** (-0.5)), 'w_uv': _w((lambda *s: _rng.normal(s) * 0.05)(Dc, H, D) * Dc ** (-0.5)), 'w_o': _w((lambda *s: _rng.normal(s) * 0.05)(H, D, M) * (H * D) ** (-0.5))}
    _B_in = _B_setup()
    return {'A_x': _A_in['x'], 'A_mem0': _A_in['mem0'], 'A_Wq': _A_in['Wq'], 'A_Wk': _A_in['Wk'], 'A_Wv': _A_in['Wv'], 'A_Wo': _A_in['Wo'], 'A_seg_len': _A_in['seg_len'], 'B_x': _B_in['x'], 'B_c_kv': _B_in['c_kv'], 'B_w_q': _B_in['w_q'], 'B_w_uk': _B_in['w_uk'], 'B_w_uv': _B_in['w_uv'], 'B_w_o': _B_in['w_o']}

def reference(A_x, A_mem0, A_Wq, A_Wk, A_Wv, A_Wo, A_seg_len, B_x, B_c_kv, B_w_q, B_w_uk, B_w_uv, B_w_o):

    def _A_ref(x, mem0, Wq, Wk, Wv, Wo, seg_len):
        B, S, Dm = x.shape
        H, Dh = (Wq.shape[1], Wq.shape[2])
        M = mem0.shape[1]
        scale = Dh ** (-0.5)
        n_seg = S // seg_len
        L = M + seg_len
        idx = jnp.arange(L)
        mask = (idx[:, None] < M) | (idx[:, None] >= idx[None, :])
        mem = mem0
        outs = []
        for s in range(n_seg):
            xs = x[:, s * seg_len:(s + 1) * seg_len, :].copy()
            h = jnp.concatenate([mem, xs], axis=1)
            q = jnp.einsum('btd,dhe->bhte', h, Wq)
            k = jnp.einsum('btd,dhe->bhte', h, Wk)
            v = jnp.einsum('btd,dhe->bhte', h, Wv)
            scores = jnp.einsum('bhqe,bhke->bhqk', q, k) * scale
            scores = jnp.where(mask[None, None], scores, -1000000000.0)
            p = _softmax(scores, axis=-1)
            o = jnp.einsum('bhqk,bhke->bhqe', p, v)
            o = jnp.einsum('bhte,hed->btd', o, Wo)
            mem = o[:, :M, :].copy()
            outs.append(o[:, M:, :])
        return jnp.concatenate(outs, axis=1)

    def _B_ref(x, c_kv, w_q, w_uk, w_uv, w_o):
        B, Sq, M = (x.shape[0], x.shape[1], x.shape[2])
        Sk = c_kv.shape[1]
        H, D = (w_q.shape[1], w_q.shape[2])
        q = jnp.einsum('bqm,mhd->bhqd', x, w_q)
        k = jnp.einsum('bkc,chd->bhkd', c_kv, w_uk)
        v = jnp.einsum('bkc,chd->bhkd', c_kv, w_uv)
        scores = jnp.einsum('bhqd,bhkd->bhqk', q, k) * D ** (-0.5)
        off = Sk - Sq
        qi = jnp.arange(Sq)[:, None]
        kj = jnp.arange(Sk)[None, :]
        cmask = kj <= qi + off
        scores = jnp.where(cmask[None, None], scores, -1000000000.0)
        p = _softmax(scores, axis=-1)
        ctx = jnp.einsum('bhqk,bhkd->bhqd', p, v)
        return jnp.einsum('bhqd,hdm->bqm', ctx, w_o)
    a = _A_ref(A_x, A_mem0, A_Wq, A_Wk, A_Wv, A_Wo, A_seg_len)
    b = _B_ref(B_x, B_c_kv, B_w_q, B_w_uk, B_w_uv, B_w_o)
    return jnp.concatenate([a, b], axis=-1)
```

```python
import math

import jax
import numpy as np
import jax.numpy as jnp
from jax.experimental import pallas as pl
from jax.experimental.pallas import tpu as pltpu

f32, bf16, u32, i32 = jnp.float32, jnp.bfloat16, jnp.uint32, jnp.int32
NT = (((1,), (1,)), ((), ()))

S, DM, DC, H, D = 2048, 448, 1024, 16, 256
NP = H // 2
NM, SEG = 8, 32
NSEG = S // SEG
MM = 384
PW = 2 * MM + 128
NK = H * (SEG + NM)
NEG = -1e30
LOG2E = math.log2(math.e)

CHAINS = 8
T = NSEG // CHAINS
R = NM * CHAINS
BQ = 256
PRB = 512
PRA = 256


def _unpack(u):
    lo = pltpu.bitcast(u << 16, f32).astype(bf16)
    hi = pltpu.bitcast(u & np.uint32(0xFFFF0000), f32).astype(bf16)
    return lo, hi


def _dot(a, b):
    return jnp.dot(a, b, preferred_element_type=f32)


def _dot_nt(a, b):
    return jax.lax.dot_general(a, b, NT, preferred_element_type=f32)


def _branch_b(xt_hbm, c_hbm, wq_hbm, wk_hbm, wv_hbm, wot_hbm, o_st, after_first_copies,
              xt, xs, cs, wq_b, wk_b, wv_b, wo_b, wq2, wkv2, q_s, k_s, v_s, acc, sems):
    wq32, wk32, wv32 = (r.bitcast(u32) for r in (wq_hbm, wk_hbm, wv_hbm))

    def copies(p, slot):
        return [pltpu.make_async_copy(wq32.at[:, p, :], wq_b.at[slot], sems.at[0, slot]),
                pltpu.make_async_copy(wk32.at[:, p, :], wk_b.at[slot], sems.at[1, slot]),
                pltpu.make_async_copy(wv32.at[:, p, :], wv_b.at[slot], sems.at[2, slot]),
                pltpu.make_async_copy(wot_hbm.at[pl.ds(2 * p, 2)], wo_b.at[slot], sems.at[3, slot])]

    cx = pltpu.make_async_copy(xt_hbm, xt, sems.at[4, 0])
    cc = pltpu.make_async_copy(c_hbm, cs, sems.at[4, 1])
    cx.start()
    cc.start()
    for c in copies(0, 0):
        c.start()
    after_first_copies()
    acc[...] = jnp.zeros_like(acc)
    cx.wait()
    xs[...] = xt[...].T
    cc.wait()
    qscale = (D ** -0.5) * LOG2E

    def pair(p, carry):
        slot = p % 2
        for c in copies(p, slot):
            c.wait()

        @pl.when(p + 1 < NP)
        def _():
            for c in copies(p + 1, 1 - slot):
                c.start()

        lo, hi = _unpack(wq_b[slot])
        wq2[0] = lo
        wq2[1] = hi
        lo, hi = _unpack(wk_b[slot])
        wkv2[0, :, 0:D] = lo
        wkv2[1, :, 0:D] = hi
        lo, hi = _unpack(wv_b[slot])
        wkv2[0, :, D:2 * D] = lo
        wkv2[1, :, D:2 * D] = hi

        def head(hh, carry):
            def proj(r, c):
                rows = pl.ds(pl.multiple_of(r * PRB, PRB), PRB)
                q_s[rows, :] = (_dot(xs[rows, :], wq2[hh]) * qscale).astype(bf16)
                kv = _dot(cs[rows, :], wkv2[hh]).astype(bf16)
                k_s[rows, :] = kv[:, 0:D]
                v_s[rows, :] = kv[:, D:2 * D]
                return c

            jax.lax.fori_loop(0, S // PRB, proj, 0)
            ri = jax.lax.broadcasted_iota(i32, (128, 128), 0)
            ci = jax.lax.broadcasted_iota(i32, (128, 128), 1)
            tri = ci <= ri
            nsub = BQ // 128
            for i in range(S // BQ):
                r0 = i * BQ
                q = q_s[r0:r0 + BQ, :]
                off = _dot_nt(q, k_s[0:r0, :]) if i > 0 else None
                strips = [_dot_nt(q[128 * a:, :], k_s[r0 + 128 * a:r0 + 128 * (a + 1), :])
                          for a in range(nsub)]
                es, ls = [], []
                for b in range(nsub):
                    parts = [off[128 * b:128 * (b + 1)]] if i > 0 else []
                    for a in range(b + 1):
                        t = strips[a][128 * (b - a):128 * (b - a + 1)]
                        parts.append(jnp.where(tri, t, NEG) if a == b else t)
                    s = jnp.concatenate(parts, axis=1) if len(parts) > 1 else parts[0]
                    m = jnp.max(s, axis=1, keepdims=True)
                    e = jnp.exp2(s - m)
                    ls.append(jnp.sum(e, axis=1, keepdims=True))
                    es.append(e.astype(bf16))
                os_ = [None] * nsub
                if i > 0:
                    o = _dot(jnp.concatenate([e[:, 0:r0] for e in es], axis=0), v_s[0:r0, :])
                for a in range(nsub):
                    c0 = r0 + 128 * a
                    oa = _dot(jnp.concatenate([e[:, c0:c0 + 128] for e in es[a:]], axis=0),
                              v_s[c0:c0 + 128, :])
                    for b in range(a, nsub):
                        t = oa[128 * (b - a):128 * (b - a + 1)]
                        os_[b] = t if os_[b] is None else os_[b] + t
                for b in range(nsub):
                    ob = os_[b] + o[128 * b:128 * (b + 1)] if i > 0 else os_[b]
                    os_[b] = (ob / ls[b]).astype(bf16)
                ctx = jnp.concatenate(os_, axis=0)
                acc[:, r0:r0 + BQ] += _dot_nt(wo_b[slot, hh], ctx)
            return carry

        jax.lax.fori_loop(0, 2, head, 0)
        return carry

    jax.lax.fori_loop(0, NP, pair, 0)
    o_st[:, DM:2 * DM] = acc[...].T.astype(bf16)


def _split_pair(z):
    rem = z[:, 2 * MM:]
    low = jax.lax.broadcasted_iota(i32, rem.shape, 1) < 64
    zero = jnp.zeros_like(rem)
    return (jnp.concatenate([z[:, 0:MM], jnp.where(low, rem, zero)], axis=1),
            jnp.concatenate([z[:, MM:2 * MM], jnp.where(low, zero, rem)], axis=1))


def _fold_rem(o):
    o3 = o[:, MM:]
    o3 = o3 + pltpu.roll(o3, 64, 1)
    return jnp.concatenate([o[:, 0:MM], o3[:, 0:DM - MM]], axis=1)


def _seg_softmax(st, mask):
    px, pm = [], []
    for h in range(H):
        sx = st[SEG * h:SEG * (h + 1), :]
        if mask is not None:
            sx = jnp.where(mask, sx, NEG)
        sm = st[H * SEG + NM * h:H * SEG + NM * (h + 1), :]
        m = jnp.maximum(jnp.max(sx, axis=0, keepdims=True), jnp.max(sm, axis=0, keepdims=True))
        ex = jnp.exp2(sx - m)
        em = jnp.exp2(sm - m)
        inv = 1.0 / (jnp.sum(ex, axis=0, keepdims=True) + jnp.sum(em, axis=0, keepdims=True))
        px.append(ex * inv)
        pm.append(em * inv)
    return jnp.concatenate(px + pm, axis=0)


def _chunk_transpose(t):
    lane = jax.lax.broadcasted_iota(i32, t[0].shape, 1)
    low = lane < 64
    even = (lane & 32) == 0
    u0 = jnp.where(low, t[0], pltpu.roll(t[2], 64, 1))
    u2 = jnp.where(low, pltpu.roll(t[0], 64, 1), t[2])
    u1 = jnp.where(low, t[1], pltpu.roll(t[3], 64, 1))
    u3 = jnp.where(low, pltpu.roll(t[1], 64, 1), t[3])
    return [jnp.where(even, u0, pltpu.roll(u1, 32, 1)), jnp.where(even, pltpu.roll(u0, 96, 1), u1),
            jnp.where(even, u2, pltpu.roll(u3, 32, 1)), jnp.where(even, pltpu.roll(u2, 96, 1), u3)]


def _branch_a(m0_ref, o_hbm, o_st, xt, wq_b, wk_b, wv_b, wo_b, sems, osem,
              xs, a4, b3, kt, v3, vm, mst):
    qscale = (D ** -0.5) * LOG2E

    def pre(p, carry):
        for j, b in enumerate((wq_b, wk_b, wv_b, wo_b)):
            pltpu.make_async_copy(b.at[p], b.at[p], sems.at[j, p]).wait()
        q0, q1 = _unpack(wq_b[p])
        k0, k1 = _unpack(wk_b[p])
        v0, v1 = _unpack(wv_b[p])
        a4[2 * p] = (_dot_nt(q0, k0) * qscale).astype(bf16)
        a4[2 * p + 1] = (_dot_nt(q1, k1) * qscale).astype(bf16)
        b0 = _dot_nt(wo_b[p, 0], v0).astype(bf16)
        b1 = _dot_nt(wo_b[p, 1], v1).astype(bf16)
        b3[p, 0:MM, :] = b0[0:MM]
        b3[p, MM:2 * MM, :] = b1[0:MM]
        b3[p, 2 * MM:2 * MM + 64, :] = b0[MM:]
        b3[p, 2 * MM + 64:, :] = b1[MM:]
        return carry

    jax.lax.fori_loop(0, NP, pre, 0)
    pltpu.make_async_copy(xt, xt, sems.at[4, 0]).wait()
    xs[...] = xt[...].T

    def proj_k(g, carry):
        for tb in range(S // 128):
            xb = xt[:, 128 * tb:128 * (tb + 1)]
            t = [pltpu.bitcast(_dot(a4[4 * g + a], xb).astype(bf16), u32) for a in range(4)]
            for b, o in enumerate(_chunk_transpose(t)):
                kt[g, 4 * tb + b] = pltpu.bitcast(o, bf16)
        return carry

    jax.lax.fori_loop(0, H // 4, proj_k, 0)

    def proj_v(i, carry):
        p = i // (S // PRA)
        rows = pl.ds(pl.multiple_of((i % (S // PRA)) * PRA, PRA), PRA)
        v3[p, rows, :] = _dot_nt(xs[rows, :], b3[p]).astype(bf16)
        return carry

    jax.lax.fori_loop(0, NP * (S // PRA), proj_v, 0)

    def keys(seg):
        return jnp.concatenate([kt[g, seg] for g in range(5)], axis=1)

    def values(seg):
        rows = pl.ds(pl.multiple_of(seg * SEG, SEG), SEG)
        hs = []
        for p in range(NP):
            hs += list(_split_pair(v3[p, rows, :]))
        return jnp.concatenate(hs + [vm[seg]], axis=0)

    m0 = m0_ref[...].astype(f32)
    mst[...] = jnp.zeros_like(mst)
    mst[0, 0:NM, :] = m0

    def step(carry):
        n, _ = carry
        j = n % T
        m = mst[j]
        mb = m.astype(bf16)
        zk = [_dot_nt(mb, a4[h]) for h in range(H)]
        for c in range(CHAINS):
            z = jnp.concatenate([zz[NM * c:NM * (c + 1)] for zz in zk], axis=0)
            kt[4, c * T + j] = z.T.astype(bf16)
        for p in range(NP):
            h0, h1 = _split_pair(_dot_nt(mb, b3[p]))
            for c in range(CHAINS):
                vm[c * T + j, 16 * p:16 * (p + 1), :] = jnp.concatenate(
                    [h0[NM * c:NM * (c + 1)], h1[NM * c:NM * (c + 1)]], axis=0).astype(bf16)
        ss = [_dot(m[NM * c:NM * (c + 1)].astype(bf16), keys(c * T + j)) for c in range(CHAINS)]
        if R < 128:
            ss.append(jnp.zeros((128 - R, NK), f32))
        pt = _seg_softmax(jnp.concatenate(ss, axis=0).T, None).T
        os_ = [_dot(pt[NM * c:NM * (c + 1)].astype(bf16), values(c * T + j)) for c in range(CHAINS)]
        new = _fold_rem(jnp.concatenate(os_, axis=0)).astype(bf16).astype(f32)
        wrap = jnp.concatenate([m0, new[0:R - NM]], axis=0) if CHAINS > 1 else m0
        jn = (n + 1) % T
        new = jnp.where(jn == 0, wrap, new)
        diff = pltpu.bitcast(new, i32) != pltpu.bitcast(mst[jn], i32)
        changed = jnp.max(diff.astype(i32))
        mst[jn] = new
        return n + 1, changed

    jax.lax.while_loop(
        lambda c: jnp.logical_and(c[0] < NSEG + T, jnp.logical_or(c[0] < T, c[1] > 0)),
        step, (jnp.int32(0), jnp.int32(1)))

    def out_copy(g):
        rows = pl.ds(pl.multiple_of(g * 128, 128), 128)
        return pltpu.make_async_copy(o_st.at[rows, :], o_hbm.at[rows, :], osem.at[g])

    def tok(g, carry):
        kk = jax.lax.broadcasted_iota(i32, (SEG, 128), 0)
        tt = jax.lax.broadcasted_iota(i32, (SEG, 128), 1) % SEG
        rows = [pl.ds(pl.multiple_of((4 * g + a) * SEG, SEG), SEG) for a in range(4)]
        ss = [_dot(xs[rows[a], :], keys(4 * g + a)) for a in range(4)]
        pt = _seg_softmax(jnp.concatenate(ss, axis=0).T, kk <= tt).T
        for a in range(4):
            o = _dot(pt[SEG * a:SEG * (a + 1)].astype(bf16), values(4 * g + a))
            o_st[rows[a], 0:DM] = _fold_rem(o).astype(bf16)
        out_copy(g).start()
        return carry

    jax.lax.fori_loop(0, NSEG // 4, tok, 0)
    for g in range(NSEG // 4):
        out_copy(g).wait()


def _kernel(axt_hbm, m0_ref, awq_hbm, awk_hbm, awv_hbm, awot_hbm,
            bxt_hbm, bc_hbm, bwq_hbm, bwk_hbm, bwv_hbm, bwot_hbm, o_hbm,
            o_st, axt, wq_b, wk_b, wv_b, wo_b, sems, osem):
    def prefetch_a():
        w32 = [r.bitcast(u32) for r in (awq_hbm, awk_hbm, awv_hbm)]
        for p in range(NP):
            for j, b in enumerate((wq_b, wk_b, wv_b)):
                pltpu.make_async_copy(w32[j].at[:, p, :], b.at[p], sems.at[j, p]).start()
            pltpu.make_async_copy(awot_hbm.at[pl.ds(2 * p, 2)], wo_b.at[p], sems.at[3, p]).start()
        pltpu.make_async_copy(axt_hbm, axt, sems.at[4, 0]).start()

    pl.run_scoped(
        lambda *s: _branch_b(bxt_hbm, bc_hbm, bwq_hbm, bwk_hbm, bwv_hbm, bwot_hbm, o_st, prefetch_a, *s),
        pltpu.VMEM((DM, S), bf16), pltpu.VMEM((S, DM), bf16), pltpu.VMEM((S, DC), bf16),
        pltpu.VMEM((2, DM, D), u32), pltpu.VMEM((2, DC, D), u32), pltpu.VMEM((2, DC, D), u32),
        pltpu.VMEM((2, 2, DM, D), bf16), pltpu.VMEM((2, DM, D), bf16), pltpu.VMEM((2, DC, 2 * D), bf16),
        pltpu.VMEM((S, D), bf16), pltpu.VMEM((S, D), bf16), pltpu.VMEM((S, D), bf16),
        pltpu.VMEM((DM, S), f32), pltpu.SemaphoreType.DMA((5, 2)))
    pl.run_scoped(
        lambda *s: _branch_a(m0_ref, o_hbm, o_st, axt, wq_b, wk_b, wv_b, wo_b, sems, osem, *s),
        pltpu.VMEM((S, DM), bf16), pltpu.VMEM((H, DM, DM), bf16), pltpu.VMEM((NP, PW, DM), bf16),
        pltpu.VMEM((5, NSEG, DM, 128), bf16), pltpu.VMEM((NP, S, PW), bf16),
        pltpu.VMEM((NSEG, 128, 512), bf16), pltpu.VMEM((T, R, DM), f32))


@jax.jit
def pallas_concat_heads__memory_aug_recurrent_mem_tr__compressed_kv_cla__prompt_kernel(
    A_x, A_mem0, A_Wq, A_Wk, A_Wv, A_Wo, A_seg_len, B_x, B_c_kv, B_w_q, B_w_uk, B_w_uv, B_w_o,
):
    del A_seg_len
    assert A_x.shape == (1, S, DM) and B_c_kv.shape == (1, S, DC) and A_Wq.shape == (DM, H, D)
    hbm = lambda a: pltpu.with_memory_space_constraint(a, pltpu.HBM)
    in_hbm = pl.BlockSpec(memory_space=pltpu.HBM)
    out = pl.pallas_call(
        _kernel,
        out_shape=pltpu.HBM((S, 2 * DM), bf16),
        in_specs=[in_hbm, pl.BlockSpec(memory_space=pltpu.VMEM)] + [in_hbm] * 10,
        out_specs=in_hbm,
        scratch_shapes=[
            pltpu.VMEM((S, 2 * DM), bf16), pltpu.VMEM((DM, S), bf16),
            pltpu.VMEM((NP, DM, D), u32), pltpu.VMEM((NP, DM, D), u32), pltpu.VMEM((NP, DM, D), u32),
            pltpu.VMEM((NP, 2, DM, D), bf16),
            pltpu.SemaphoreType.DMA((5, NP)), pltpu.SemaphoreType.DMA((NSEG // 4,))],
        compiler_params=pltpu.CompilerParams(vmem_limit_bytes=120 * 1024 * 1024),
        name="fused_rmt_mla",
    )(hbm(A_x[0].T), A_mem0[0], hbm(A_Wq), hbm(A_Wk), hbm(A_Wv), hbm(A_Wo.transpose(0, 2, 1)),
      hbm(B_x[0].T), hbm(B_c_kv[0]), hbm(B_w_q), hbm(B_w_uk), hbm(B_w_uv), hbm(B_w_o.transpose(0, 2, 1)))
    return out[None]
```

```python
import math

import jax
import numpy as np
import jax.numpy as jnp
from jax.experimental import pallas as pl
from jax.experimental.pallas import tpu as pltpu

f32, bf16, u32, i32 = jnp.float32, jnp.bfloat16, jnp.uint32, jnp.int32
NT = (((1,), (1,)), ((), ()))

S, DM, DC, H, D = 2048, 448, 1024, 16, 256
NP = H // 2
NM, SEG = 8, 32
NSEG = S // SEG
MM = 384
PW = 2 * MM + 128
NK = H * (SEG + NM)
NEG = -1e30
LOG2E = math.log2(math.e)

CHAINS = 8
T = NSEG // CHAINS
R = NM * CHAINS
import os
BQ = int(os.environ.get('BQ', 256))
CK = 256
PRB = int(os.environ.get('PRB', 512))
PRA = 512


def _unpack(u):
    lo = pltpu.bitcast(u << 16, f32).astype(bf16)
    hi = pltpu.bitcast(u & np.uint32(0xFFFF0000), f32).astype(bf16)
    return lo, hi


def _dot(a, b):
    return jnp.dot(a, b, preferred_element_type=f32)


def _dot_nt(a, b):
    return jax.lax.dot_general(a, b, NT, preferred_element_type=f32)


def _branch_b(xt_hbm, c_hbm, wq_hbm, wk_hbm, wv_hbm, wot_hbm, prefetch_a,
              xt, xs, cs, wq_b, wk_b, wv_b, wo_b, wq1, wkv1, q_s, k_s, v_s, acc, sems, csem):
    wq32, wk32, wv32 = (r.bitcast(u32) for r in (wq_hbm, wk_hbm, wv_hbm))
    nsub, nq = BQ // 128, S // BQ

    def copies(p, slot):
        return [pltpu.make_async_copy(wq32.at[:, p, :], wq_b.at[slot], sems.at[0, slot]),
                pltpu.make_async_copy(wk32.at[:, p, :], wk_b.at[slot], sems.at[1, slot]),
                pltpu.make_async_copy(wv32.at[:, p, :], wv_b.at[slot], sems.at[2, slot]),
                pltpu.make_async_copy(wot_hbm.at[pl.ds(2 * p, 2)], wo_b.at[slot], sems.at[3, slot])]

    def c_copy(r):
        rows = pl.ds(r * PRB, PRB)
        return pltpu.make_async_copy(c_hbm.at[rows, :], cs.at[rows, :], csem.at[r])

    def prepare(h, r, n, which=(0, 1, 2)):
        slot, dst = (h // 2) % 2, h % 2
        sh = np.uint32(16 * (1 - h % 2)) if isinstance(h, int) else (16 * (1 - h % 2)).astype(u32)
        half = lambda u: pltpu.bitcast((u << sh) & np.uint32(0xFFFF0000), f32).astype(bf16)
        rq = pl.ds(r * (DM // n), DM // n)
        rc = pl.ds(r * (DC // n), DC // n)
        if 0 in which:
            wq1[dst, rq, :] = half(wq_b[slot, rq, :])
        if 1 in which:
            wkv1[dst, rc, 0:D] = half(wk_b[slot, rc, :])
        if 2 in which:
            wkv1[dst, rc, D:2 * D] = half(wv_b[slot, rc, :])

    cx = pltpu.make_async_copy(xt_hbm, xt, sems.at[4, 0])
    cx.start()
    first = copies(0, 0)
    for c in first[:3]:
        c.start()
    for r in range(S // PRB):
        c_copy(r).start()
    first[3].start()
    acc[...] = jnp.zeros_like(acc)
    cx.wait()
    xs[...] = xt[...].T
    for j in range(3):
        first[j].wait()
        prepare(0, 0, 1, (j,))
    qscale = (D ** -0.5) * LOG2E

    ri = jax.lax.broadcasted_iota(i32, (128, 128), 0)
    ci = jax.lax.broadcasted_iota(i32, (128, 128), 1)
    tri = ci <= ri

    def scores(i):
        r0 = i * BQ
        q = q_s[r0:r0 + BQ, :]
        chunks = [_dot_nt(q, k_s[c0:c0 + CK, :]) for c0 in range(0, r0, CK)]
        strips = []
        for a in range(nsub):
            t = _dot_nt(q[128 * a:, :], k_s[r0 + 128 * a:r0 + 128 * (a + 1), :])
            top = jnp.where(tri, t[0:128], NEG)
            strips.append(jnp.concatenate([top, t[128:]], axis=0) if a + 1 < nsub else top)
        return chunks, strips

    def attend(i, chunks, strips):
        r0 = i * BQ
        ms = []
        for b in range(nsub):
            parts = [t[128 * b:128 * (b + 1)] for t in chunks]
            parts += [strips[a][128 * (b - a):128 * (b - a + 1)] for a in range(b + 1)]
            ms.append(jnp.max(jnp.concatenate(parts, axis=1), axis=1, keepdims=True))
        m = jnp.concatenate(ms, axis=0)
        o = l = None
        for c, t in enumerate(chunks):
            e = jnp.exp2(t - m)
            for u in range(0, CK, 128):
                l = e[:, u:u + 128] if l is None else l + e[:, u:u + 128]
            pv = _dot(e.astype(bf16), v_s[c * CK:(c + 1) * CK, :])
            o = pv if o is None else o + pv
        os_ = [None if o is None else o[128 * b:128 * (b + 1)] for b in range(nsub)]
        ls = [None if l is None else l[128 * b:128 * (b + 1)] for b in range(nsub)]
        for a in range(nsub):
            e = jnp.exp2(strips[a] - m[128 * a:])
            pv = _dot(e.astype(bf16), v_s[r0 + 128 * a:r0 + 128 * (a + 1), :])
            for b in range(a, nsub):
                sl = slice(128 * (b - a), 128 * (b - a + 1))
                os_[b] = pv[sl] if os_[b] is None else os_[b] + pv[sl]
                ls[b] = e[sl] if ls[b] is None else ls[b] + e[sl]
        return jnp.concatenate(os_, axis=0), jnp.concatenate(ls, axis=0)

    def head(h, carry):
        p = h // 2

        @pl.when(jnp.logical_and(h % 2 == 1, h + 1 < H))
        def _():
            for c in copies(p + 1, (p + 1) % 2):
                c.wait()

        @pl.when(h == 0)
        def _():
            for r in range(S // PRB):
                c_copy(r).wait()
            first[3].wait()
            for c in copies(1, 1):
                c.start()

        @pl.when(h == 2)
        def _():
            prefetch_a()

        for r in range(S // PRB):
            rows = pl.ds(r * PRB, PRB)
            prepare(h + 1, r, S // PRB)
            q_s[rows, :] = (_dot(xs[rows, :], wq1[h % 2]) * qscale).astype(bf16)
            kv = _dot(cs[rows, :], wkv1[h % 2]).astype(bf16)
            k_s[rows, :] = kv[:, 0:D]
            v_s[rows, :] = kv[:, D:2 * D]

        def project_out(i, o, l):
            ctx = (o * (1.0 / jnp.sum(l, axis=1, keepdims=True))).astype(bf16)
            acc[:, i * BQ:(i + 1) * BQ] += _dot_nt(wo_b[p % 2, h % 2], ctx)

        cur, prev = scores(nq - 1), None
        for i in reversed(range(nq)):
            nxt = scores(i - 1) if i > 0 else None
            new = attend(i, *cur)
            if prev is not None:
                project_out(i + 1, *prev)
            cur, prev = nxt, new
        project_out(0, *prev)

        @pl.when(jnp.logical_and(h % 2 == 1, p + 2 < NP))
        def _():
            for c in copies(p + 2, p % 2):
                c.start()

        return carry

    jax.lax.fori_loop(0, H, head, 0)


def _split_pair(z):
    rem = z[:, 2 * MM:]
    bits = rem if rem.dtype == f32 else pltpu.bitcast(rem, u32)
    low = jax.lax.broadcasted_iota(i32, bits.shape, 1) < 64
    zero = jnp.zeros_like(bits)
    r0, r1 = jnp.where(low, bits, zero), jnp.where(low, zero, bits)
    if rem.dtype != f32:
        r0, r1 = pltpu.bitcast(r0, rem.dtype), pltpu.bitcast(r1, rem.dtype)
    return (jnp.concatenate([z[:, 0:MM], r0], axis=1), jnp.concatenate([z[:, MM:2 * MM], r1], axis=1))


def _fold_rem(o):
    o3 = o[:, MM:]
    o3 = o3 + pltpu.roll(o3, 64, 1)
    return jnp.concatenate([o[:, 0:MM], o3[:, 0:DM - MM]], axis=1)


def _seg_softmax(st, mask):
    px, pm = [], []
    for h in range(H):
        sx = st[SEG * h:SEG * (h + 1), :]
        if mask is not None:
            sx = jnp.where(mask, sx, NEG)
        sm = st[H * SEG + NM * h:H * SEG + NM * (h + 1), :]
        m = jnp.maximum(jnp.max(sx, axis=0, keepdims=True), jnp.max(sm, axis=0, keepdims=True))
        ex = jnp.exp2(sx - m)
        em = jnp.exp2(sm - m)
        inv = 1.0 / (jnp.sum(ex, axis=0, keepdims=True) + jnp.sum(em, axis=0, keepdims=True))
        px.append(ex * inv)
        pm.append(em * inv)
    return jnp.concatenate(px + pm, axis=0)


def _chunk_transpose(t):
    lane = jax.lax.broadcasted_iota(i32, t[0].shape, 1)
    low = lane < 64
    even = (lane & 32) == 0
    u0 = jnp.where(low, t[0], pltpu.roll(t[2], 64, 1))
    u2 = jnp.where(low, pltpu.roll(t[0], 64, 1), t[2])
    u1 = jnp.where(low, t[1], pltpu.roll(t[3], 64, 1))
    u3 = jnp.where(low, pltpu.roll(t[1], 64, 1), t[3])
    return [jnp.where(even, u0, pltpu.roll(u1, 32, 1)), jnp.where(even, pltpu.roll(u0, 96, 1), u1),
            jnp.where(even, u2, pltpu.roll(u3, 32, 1)), jnp.where(even, pltpu.roll(u2, 96, 1), u3)]


def _absorb(wq_b, wk_b, wv_b, wo_b, sems, a3, b3, acc, o_st, xt, xs):
    qscale = (D ** -0.5) * LOG2E
    pltpu.make_async_copy(xt, xt, sems.at[4, 0]).wait()

    def pre(p, carry):
        for j, b in enumerate((wq_b, wk_b, wv_b, wo_b)):
            pltpu.make_async_copy(b.at[p], b.at[p], sems.at[j, p]).wait()
        q, k, v = _unpack(wq_b[p]), _unpack(wk_b[p]), _unpack(wv_b[p])
        for u in range(2):
            for dst, w in ((a3, _dot_nt(q[u], k[u]) * qscale), (b3, _dot_nt(wo_b[p, u], v[u]))):
                w = w.astype(bf16)
                dst[p, u * MM:(u + 1) * MM, :] = w[0:MM]
                dst[p, 2 * MM + 64 * u:2 * MM + 64 * (u + 1), :] = w[MM:]
        tok = pl.ds(pl.multiple_of(p * (S // NP), S // NP), S // NP)
        o_st[tok, DM:2 * DM] = acc[:, tok].astype(bf16).T
        xs[tok, :] = xt[:, tok].T
        return carry

    jax.lax.fori_loop(0, NP, pre, 0)


def _branch_a(m0_ref, o_hbm, o_st, xt, xs, a3, b3, osem, kt, v3, vm, mst):
    def proj_k(g, carry):
        for tb in range(S // 128):
            xb = xt[:, 128 * tb:128 * (tb + 1)]
            t = []
            for pp in range(2):
                z = _dot(a3[2 * g + pp], xb).astype(bf16)
                for u in range(2):
                    t.append(pltpu.bitcast(jnp.concatenate(
                        [z[u * MM:(u + 1) * MM], z[2 * MM + 64 * u:2 * MM + 64 * (u + 1)]], axis=0), u32))
            for b, o in enumerate(_chunk_transpose(t)):
                kt[g, 4 * tb + b] = pltpu.bitcast(o, bf16)
        return carry

    jax.lax.fori_loop(0, H // 4, proj_k, 0)

    def proj_v(p, carry):
        for r in range(S // PRA):
            rows = pl.ds(r * PRA, PRA)
            v3[p, rows, :] = _dot_nt(xs[rows, :], b3[p]).astype(bf16)
        return carry

    jax.lax.fori_loop(0, NP, proj_v, 0)

    def keys(seg):
        return jnp.concatenate([kt[g, seg] for g in range(5)], axis=1)

    def values(seg):
        rows = pl.ds(seg * SEG if isinstance(seg, int) else pl.multiple_of(seg * SEG, SEG), SEG)
        hs = []
        for p in range(NP):
            hs += list(_split_pair(v3[p, rows, :]))
        return jnp.concatenate(hs + [vm[seg]], axis=0)

    m0 = m0_ref[...].astype(f32)
    mst[...] = jnp.zeros_like(mst)
    mst[0, 0:NM, :] = m0

    def step(carry):
        n, _ = carry
        j = n % T
        m = mst[j]
        mb = m.astype(bf16)
        zk = [_dot_nt(mb, a3[p]) for p in range(NP)]
        even = (jax.lax.broadcasted_iota(i32, (32, 128), 1) & NM) == 0
        for c in range(CHAINS):
            cr = slice(NM * c, NM * (c + 1))
            z = jnp.concatenate(
                [jnp.concatenate([zz[cr, u * MM:(u + 1) * MM], zz[cr, 2 * MM:]], axis=1)
                 for zz in zk for u in range(2)], axis=0).astype(bf16).T
            kt[4, c * T + j, 0:MM, :] = z[0:MM]
            kt[4, c * T + j, MM:, :] = pltpu.bitcast(
                jnp.where(even, pltpu.bitcast(z[MM:MM + 64], u32), pltpu.bitcast(z[MM + 64:], u32)), bf16)
        for p in range(NP):
            h0, h1 = _split_pair(_dot_nt(mb, b3[p]))
            for c in range(CHAINS):
                vm[c * T + j, 16 * p:16 * (p + 1), :] = jnp.concatenate(
                    [h0[NM * c:NM * (c + 1)], h1[NM * c:NM * (c + 1)]], axis=0).astype(bf16)
        ss = [_dot(m[NM * c:NM * (c + 1)].astype(bf16), keys(c * T + j)) for c in range(CHAINS)]
        if R < 128:
            ss.append(jnp.zeros((128 - R, NK), f32))
        pt = _seg_softmax(jnp.concatenate(ss, axis=0).T, None).T
        os_ = [_dot(pt[NM * c:NM * (c + 1)].astype(bf16), values(c * T + j)) for c in range(CHAINS)]
        new = _fold_rem(jnp.concatenate(os_, axis=0)).astype(bf16).astype(f32)
        wrap = jnp.concatenate([m0, new[0:R - NM]], axis=0) if CHAINS > 1 else m0
        jn = (n + 1) % T
        new = jnp.where(jn == 0, wrap, new)
        diff = pltpu.bitcast(new, i32) != pltpu.bitcast(mst[jn], i32)
        changed = jnp.max(diff.astype(i32))
        mst[jn] = new
        return n + 1, changed

    jax.lax.while_loop(
        lambda c: jnp.logical_and(c[0] < NSEG + T, jnp.logical_or(c[0] < T, c[1] > 0)),
        step, (jnp.int32(0), jnp.int32(1)))

    def out_copy(g):
        rows = pl.ds(g * 128, 128)
        return pltpu.make_async_copy(o_st.at[rows, :], o_hbm.at[rows, :], osem.at[g])

    kk = jax.lax.broadcasted_iota(i32, (SEG, 128), 0)
    tt = jax.lax.broadcasted_iota(i32, (SEG, 128), 1) % SEG
    ng = NSEG // 4
    cur = None
    for g in range(ng + 1):
        nxt = None
        if g < ng:
            nxt = jnp.concatenate(
                [_dot(xs[(4 * g + a) * SEG:(4 * g + a + 1) * SEG, :], keys(4 * g + a)) for a in range(4)], axis=0)
        if cur is not None:
            pt = _seg_softmax(cur.T, kk <= tt).T
            for a in range(4):
                seg = 4 * (g - 1) + a
                o = _dot(pt[SEG * a:SEG * (a + 1)].astype(bf16), values(seg))
                o_st[seg * SEG:(seg + 1) * SEG, 0:DM] = _fold_rem(o).astype(bf16)
            out_copy(g - 1).start()
        cur = nxt
    for g in range(ng):
        out_copy(g).wait()


def _kernel(axt_hbm, m0_ref, awq_hbm, awk_hbm, awv_hbm, awot_hbm,
            bxt_hbm, bc_hbm, bwq_hbm, bwk_hbm, bwv_hbm, bwot_hbm, o_hbm,
            o_st, axt, axs, a3, b3, osem):
    def phase1(wq_b, wk_b, wv_b, wo_b, sems, acc, *s):
        def prefetch_a():
            w32 = [r.bitcast(u32) for r in (awq_hbm, awk_hbm, awv_hbm)]
            for p in range(NP):
                for j, b in enumerate((wq_b, wk_b, wv_b)):
                    pltpu.make_async_copy(w32[j].at[:, p, :], b.at[p], sems.at[j, p]).start()
                pltpu.make_async_copy(awot_hbm.at[pl.ds(2 * p, 2)], wo_b.at[p], sems.at[3, p]).start()
            pltpu.make_async_copy(axt_hbm, axt, sems.at[4, 0]).start()

        _branch_b(bxt_hbm, bc_hbm, bwq_hbm, bwk_hbm, bwv_hbm, bwot_hbm, prefetch_a, *s[:-2], acc, *s[-2:])
        _absorb(wq_b, wk_b, wv_b, wo_b, sems, a3, b3, acc, o_st, axt, axs)

    pl.run_scoped(
        phase1,
        pltpu.VMEM((NP, DM, D), u32), pltpu.VMEM((NP, DM, D), u32), pltpu.VMEM((NP, DM, D), u32),
        pltpu.VMEM((NP, 2, DM, D), bf16), pltpu.SemaphoreType.DMA((5, NP)), pltpu.VMEM((DM, S), f32),
        pltpu.VMEM((DM, S), bf16), pltpu.VMEM((S, DM), bf16), pltpu.VMEM((S, DC), bf16),
        pltpu.VMEM((2, DM, D), u32), pltpu.VMEM((2, DC, D), u32), pltpu.VMEM((2, DC, D), u32),
        pltpu.VMEM((2, 2, DM, D), bf16), pltpu.VMEM((2, DM, D), bf16), pltpu.VMEM((2, DC, 2 * D), bf16),
        pltpu.VMEM((S, D), bf16), pltpu.VMEM((S, D), bf16), pltpu.VMEM((S, D), bf16),
        pltpu.SemaphoreType.DMA((5, 2)), pltpu.SemaphoreType.DMA((S // PRB,)))
    pl.run_scoped(
        lambda *s: _branch_a(m0_ref, o_hbm, o_st, axt, axs, a3, b3, osem, *s),
        pltpu.VMEM((5, NSEG, DM, 128), bf16), pltpu.VMEM((NP, S, PW), bf16),
        pltpu.VMEM((NSEG, 128, 512), bf16), pltpu.VMEM((T, R, DM), f32))


@jax.jit
def pallas_concat_heads__memory_aug_recurrent_mem_tr__compressed_kv_cla__prompt_kernel(
    A_x, A_mem0, A_Wq, A_Wk, A_Wv, A_Wo, A_seg_len, B_x, B_c_kv, B_w_q, B_w_uk, B_w_uv, B_w_o,
):
    del A_seg_len
    assert A_x.shape == (1, S, DM) and B_c_kv.shape == (1, S, DC) and A_Wq.shape == (DM, H, D)
    hbm = lambda a: pltpu.with_memory_space_constraint(a, pltpu.HBM)
    in_hbm = pl.BlockSpec(memory_space=pltpu.HBM)
    out = pl.pallas_call(
        _kernel,
        out_shape=pltpu.HBM((S, 2 * DM), bf16),
        in_specs=[in_hbm, pl.BlockSpec(memory_space=pltpu.VMEM)] + [in_hbm] * 10,
        out_specs=in_hbm,
        scratch_shapes=[
            pltpu.VMEM((S, 2 * DM), bf16), pltpu.VMEM((DM, S), bf16), pltpu.VMEM((S, DM), bf16),
            pltpu.VMEM((NP, PW, DM), bf16), pltpu.VMEM((NP, PW, DM), bf16),
            pltpu.SemaphoreType.DMA((NSEG // 4,))],
        compiler_params=pltpu.CompilerParams(vmem_limit_bytes=120 * 1024 * 1024),
        name="fused_rmt_mla",
    )(hbm(A_x[0].T), A_mem0[0], hbm(A_Wq), hbm(A_Wk), hbm(A_Wv), hbm(A_Wo.transpose(0, 2, 1)),
      hbm(B_x[0].T), hbm(B_c_kv[0]), hbm(B_w_q), hbm(B_w_uk), hbm(B_w_uv), hbm(B_w_o.transpose(0, 2, 1)))
    return out[None]
```

```python
import functools
import math

import jax
import numpy as np
import jax.numpy as jnp
from jax.experimental import pallas as pl
from jax.experimental.pallas import tpu as pltpu

f32, bf16, u32, i32 = jnp.float32, jnp.bfloat16, jnp.uint32, jnp.int32
NT = (((1,), (1,)), ((), ()))

S, DM, DC, H, D = 2048, 448, 1024, 16, 256
NP = H // 2
NM, SEG = 8, 32
NSEG = S // SEG
MM = 384
PW = 2 * MM + 128
NK = H * (SEG + NM)
NEG = -1e30
LOG2E = math.log2(math.e)

CHAINS = 8
T = NSEG // CHAINS
R = NM * CHAINS
import os
BQ = int(os.environ.get('BQ', 256))
CK = 256
PRB = int(os.environ.get('PRB', 512))
PRA = 512


def _half(w, u):
    sh = np.uint32(16 * (1 - u)) if isinstance(u, int) else (16 * (1 - u)).astype(u32)
    return pltpu.bitcast((w << sh) & np.uint32(0xFFFF0000), f32).astype(bf16)


def _dot(a, b):
    return jnp.dot(a, b, preferred_element_type=f32)


def _dot_nt(a, b):
    return jax.lax.dot_general(a, b, NT, preferred_element_type=f32)


def _branch_b(xt_hbm, c_hbm, wq_hbm, wk_hbm, wv_hbm, wot_hbm, acc, overlapped_work,
              xt, xs, cs, wq_b, wk_b, wv_b, wo_b, wq1, wkv1, q_s, k_s, v_s, sems):
    wq32, wk32, wv32 = (r.bitcast(u32) for r in (wq_hbm, wk_hbm, wv_hbm))
    nsub, nq = BQ // 128, S // BQ

    def copies(p, slot):
        return [pltpu.make_async_copy(wq32.at[:, p, :], wq_b.at[slot], sems.at[0, slot]),
                pltpu.make_async_copy(wk32.at[:, p, :], wk_b.at[slot], sems.at[1, slot]),
                pltpu.make_async_copy(wv32.at[:, p, :], wv_b.at[slot], sems.at[2, slot]),
                pltpu.make_async_copy(wot_hbm.at[pl.ds(2 * p, 2)], wo_b.at[slot], sems.at[3, slot])]

    def prepare(h, r, n):
        slot, dst = (h // 2) % 2, h % 2
        half = lambda w: _half(w, h % 2)
        part = lambda w: pl.ds(r * w if isinstance(r, int) else pl.multiple_of(r * w, w), w)
        rq, rc = part(DM // n), part(DC // n)
        wq1[dst, rq, :] = half(wq_b[slot, rq, :])
        wkv1[dst, rc, 0:D] = half(wk_b[slot, rc, :])
        wkv1[dst, rc, D:2 * D] = half(wv_b[slot, rc, :])

    cx = pltpu.make_async_copy(xt_hbm, xt, sems.at[4, 0])
    cc = pltpu.make_async_copy(c_hbm, cs, sems.at[4, 1])
    for c in [cx, cc] + copies(0, 0) + copies(1, 1):
        c.start()
    overlapped_work()
    for c in [cx, cc] + copies(0, 0):
        c.wait()

    def first(r, carry):
        rows = pl.ds(pl.multiple_of(r * PRB, PRB), PRB)
        xs[rows, :] = xt[:, rows].T
        acc[:, rows] = jnp.zeros((DM, PRB), f32)
        prepare(0, r, S // PRB)
        return carry

    jax.lax.fori_loop(0, S // PRB, first, 0)
    qscale = (D ** -0.5) * LOG2E

    ri = jax.lax.broadcasted_iota(i32, (128, 128), 0)
    ci = jax.lax.broadcasted_iota(i32, (128, 128), 1)
    tri = ci <= ri

    def scores(i):
        r0 = i * BQ
        q = q_s[r0:r0 + BQ, :]
        chunks = [_dot_nt(q, k_s[c0:c0 + CK, :]) for c0 in range(0, r0, CK)]
        strips = []
        for a in range(nsub):
            t = _dot_nt(q[128 * a:, :], k_s[r0 + 128 * a:r0 + 128 * (a + 1), :])
            top = jnp.where(tri, t[0:128], NEG)
            strips.append(jnp.concatenate([top, t[128:]], axis=0) if a + 1 < nsub else top)
        return chunks, strips

    def attend(i, chunks, strips):
        r0 = i * BQ
        ms = []
        for b in range(nsub):
            parts = [t[128 * b:128 * (b + 1)] for t in chunks]
            parts += [strips[a][128 * (b - a):128 * (b - a + 1)] for a in range(b + 1)]
            ms.append(jnp.max(jnp.concatenate(parts, axis=1), axis=1, keepdims=True))
        m = jnp.concatenate(ms, axis=0)
        o = l = None
        for c, t in enumerate(chunks):
            e = jnp.exp2(t - m)
            for u in range(0, CK, 128):
                l = e[:, u:u + 128] if l is None else l + e[:, u:u + 128]
            pv = _dot(e.astype(bf16), v_s[c * CK:(c + 1) * CK, :])
            o = pv if o is None else o + pv
        os_ = [None if o is None else o[128 * b:128 * (b + 1)] for b in range(nsub)]
        ls = [None if l is None else l[128 * b:128 * (b + 1)] for b in range(nsub)]
        for a in range(nsub):
            e = jnp.exp2(strips[a] - m[128 * a:])
            pv = _dot(e.astype(bf16), v_s[r0 + 128 * a:r0 + 128 * (a + 1), :])
            for b in range(a, nsub):
                sl = slice(128 * (b - a), 128 * (b - a + 1))
                os_[b] = pv[sl] if os_[b] is None else os_[b] + pv[sl]
                ls[b] = e[sl] if ls[b] is None else ls[b] + e[sl]
        return jnp.concatenate(os_, axis=0), jnp.concatenate(ls, axis=0)

    def head(h, carry):
        p = h // 2

        @pl.when(jnp.logical_and(h % 2 == 1, h + 1 < H))
        def _():
            for c in copies(p + 1, (p + 1) % 2):
                c.wait()

        for r in range(S // PRB):
            rows = pl.ds(r * PRB, PRB)
            prepare(h + 1, r, S // PRB)
            q_s[rows, :] = (_dot(xs[rows, :], wq1[h % 2]) * qscale).astype(bf16)
            kv = _dot(cs[rows, :], wkv1[h % 2]).astype(bf16)
            k_s[rows, :] = kv[:, 0:D]
            v_s[rows, :] = kv[:, D:2 * D]

        def project_out(i, o, l):
            ctx = (o * (1.0 / jnp.sum(l, axis=1, keepdims=True))).astype(bf16)
            acc[:, i * BQ:(i + 1) * BQ] += _dot_nt(wo_b[p % 2, h % 2], ctx)

        cur, prev = scores(nq - 1), None
        for i in reversed(range(nq)):
            nxt = scores(i - 1) if i > 0 else None
            new = attend(i, *cur)
            if prev is not None:
                project_out(i + 1, *prev)
            cur, prev = nxt, new
        project_out(0, *prev)

        @pl.when(jnp.logical_and(h % 2 == 1, p + 2 < NP))
        def _():
            for c in copies(p + 2, p % 2):
                c.start()

        return carry

    jax.lax.fori_loop(0, H, head, 0)


def _split_pair(z):
    rem = z[:, 2 * MM:]
    bits = rem if rem.dtype == f32 else pltpu.bitcast(rem, u32)
    low = jax.lax.broadcasted_iota(i32, bits.shape, 1) < 64
    zero = jnp.zeros_like(bits)
    r0, r1 = jnp.where(low, bits, zero), jnp.where(low, zero, bits)
    if rem.dtype != f32:
        r0, r1 = pltpu.bitcast(r0, rem.dtype), pltpu.bitcast(r1, rem.dtype)
    return (jnp.concatenate([z[:, 0:MM], r0], axis=1), jnp.concatenate([z[:, MM:2 * MM], r1], axis=1))


def _fold_rem(o):
    o3 = o[:, MM:]
    o3 = o3 + pltpu.roll(o3, 64, 1)
    return jnp.concatenate([o[:, 0:MM], o3[:, 0:DM - MM]], axis=1)


def _seg_softmax(st, mask):
    px, pm = [], []
    for h in range(H):
        sx = st[SEG * h:SEG * (h + 1), :]
        if mask is not None:
            sx = jnp.where(mask, sx, NEG)
        sm = st[H * SEG + NM * h:H * SEG + NM * (h + 1), :]
        m = jnp.maximum(jnp.max(sx, axis=0, keepdims=True), jnp.max(sm, axis=0, keepdims=True))
        ex = jnp.exp2(sx - m)
        em = jnp.exp2(sm - m)
        inv = 1.0 / (jnp.sum(ex, axis=0, keepdims=True) + jnp.sum(em, axis=0, keepdims=True))
        px.append(ex * inv)
        pm.append(em * inv)
    return jnp.concatenate(px + pm, axis=0)


def _chunk_transpose(t):
    lane = jax.lax.broadcasted_iota(i32, t[0].shape, 1)
    low = lane < 64
    even = (lane & 32) == 0
    u0 = jnp.where(low, t[0], pltpu.roll(t[2], 64, 1))
    u2 = jnp.where(low, pltpu.roll(t[0], 64, 1), t[2])
    u1 = jnp.where(low, t[1], pltpu.roll(t[3], 64, 1))
    u3 = jnp.where(low, pltpu.roll(t[1], 64, 1), t[3])
    return [jnp.where(even, u0, pltpu.roll(u1, 32, 1)), jnp.where(even, pltpu.roll(u0, 96, 1), u1),
            jnp.where(even, u2, pltpu.roll(u3, 32, 1)), jnp.where(even, pltpu.roll(u2, 96, 1), u3)]


def _absorb(wq_hbm, wk_hbm, wv_hbm, wot_hbm, xt_copy, a3, b3, wq_b, wk_b, wv_b, wo_b, sems):
    qscale = (D ** -0.5) * LOG2E
    w32 = [r.bitcast(u32) for r in (wq_hbm, wk_hbm, wv_hbm)]

    def copies(p):
        cs = [pltpu.make_async_copy(w32[j].at[:, p, :], b.at[p], sems.at[j, p])
              for j, b in enumerate((wq_b, wk_b, wv_b))]
        return cs + [pltpu.make_async_copy(wot_hbm.at[pl.ds(2 * p, 2)], wo_b.at[p], sems.at[3, p])]

    for c in copies(0) + copies(1):
        c.start()

    def pre(h, carry):
        p, u = h // 2, h % 2

        @pl.when(u == 0)
        def _():
            for c in copies(p):
                c.wait()

            @pl.when(p + 2 < NP)
            def _():
                for c in copies(p + 2):
                    c.start()

            @pl.when(p + 2 == NP)
            def _():
                xt_copy.start()

        q, k, v = (_half(b[p], u) for b in (wq_b, wk_b, wv_b))
        for dst, w in ((a3, _dot_nt(q, k) * qscale), (b3, _dot_nt(wo_b[p, u], v))):
            w = w.astype(bf16)
            dst[p, pl.ds(pl.multiple_of(u * MM, MM), MM), :] = w[0:MM]
            dst[p, pl.ds(pl.multiple_of(2 * MM + 64 * u, 64), 64), :] = w[MM:]
        return carry

    jax.lax.fori_loop(0, H, pre, 0)
    xt_copy.wait()


def _project_keys(xt, xs, a3, kt):
    nb = PRA // 128

    def proj_k(i, carry):
        g, t0 = i // (S // PRA), (i % (S // PRA)) * nb
        tok = pl.ds(pl.multiple_of(i * 128, 128), 128)
        xs[tok, :] = xt[:, tok].T
        for tb in range(nb):
            xb = xt[:, pl.ds(pl.multiple_of((t0 + tb) * 128, 128), 128)]
            t = []
            for pp in range(2):
                z = _dot(a3[2 * g + pp], xb).astype(bf16)
                for u in range(2):
                    t.append(pltpu.bitcast(jnp.concatenate(
                        [z[u * MM:(u + 1) * MM], z[2 * MM + 64 * u:2 * MM + 64 * (u + 1)]], axis=0), u32))
            for b, o in enumerate(_chunk_transpose(t)):
                kt[g, 4 * (t0 + tb) + b] = pltpu.bitcast(o, bf16)
        return carry

    jax.lax.fori_loop(0, (H // 4) * (S // PRA), proj_k, 0)


def _branch_a(m0_ref, o_hbm, acc, xs, a3, b3, kt, o_st, v3, vm, mst, ssc, osem):
    def proj_v(i, carry):
        p = i // 2
        tok = pl.ds(pl.multiple_of(i * 128, 128), 128)
        o_st[tok, DM:2 * DM] = acc[:, tok].astype(bf16).T
        for r in range(S // PRA // 2):
            rows = pl.ds(pl.multiple_of((i % 2) * (S // 2) + r * PRA, PRA), PRA)
            v3[p, rows, :] = _dot_nt(xs[rows, :], b3[p]).astype(bf16)
        return carry

    jax.lax.fori_loop(0, 2 * NP, proj_v, 0)

    def keys(seg):
        return jnp.concatenate([kt[g, seg] for g in range(5)], axis=1)

    def values(seg):
        rows = pl.ds(pl.multiple_of(seg * SEG, SEG), SEG)
        hs = []
        for p in range(NP):
            hs += list(_split_pair(v3[p, rows, :]))
        return jnp.concatenate(hs + [vm[seg]], axis=0)

    m0 = m0_ref[...].astype(f32)
    mst[...] = jnp.zeros_like(mst)
    mst[0, 0:NM, :] = m0

    def step(carry):
        n, _ = carry
        j = n % T
        m = mst[j]
        mb = m.astype(bf16)
        zk = [_dot_nt(mb, a3[p]) for p in range(NP)]
        even = (jax.lax.broadcasted_iota(i32, (32, 128), 1) & NM) == 0
        for c in range(CHAINS):
            cr = slice(NM * c, NM * (c + 1))
            z = jnp.concatenate(
                [jnp.concatenate([zz[cr, u * MM:(u + 1) * MM], zz[cr, 2 * MM:]], axis=1)
                 for zz in zk for u in range(2)], axis=0).astype(bf16).T
            kt[4, c * T + j, 0:MM, :] = z[0:MM]
            kt[4, c * T + j, MM:, :] = pltpu.bitcast(
                jnp.where(even, pltpu.bitcast(z[MM:MM + 64], u32), pltpu.bitcast(z[MM + 64:], u32)), bf16)
        for p in range(NP):
            h0, h1 = _split_pair(_dot_nt(mb, b3[p]))
            for c in range(CHAINS):
                vm[c * T + j, 16 * p:16 * (p + 1), :] = jnp.concatenate(
                    [h0[NM * c:NM * (c + 1)], h1[NM * c:NM * (c + 1)]], axis=0).astype(bf16)
        ss = [_dot(m[NM * c:NM * (c + 1)].astype(bf16), keys(c * T + j)) for c in range(CHAINS)]
        if R < 128:
            ss.append(jnp.zeros((128 - R, NK), f32))
        pt = _seg_softmax(jnp.concatenate(ss, axis=0).T, None).T
        os_ = [_dot(pt[NM * c:NM * (c + 1)].astype(bf16), values(c * T + j)) for c in range(CHAINS)]
        new = _fold_rem(jnp.concatenate(os_, axis=0)).astype(bf16).astype(f32)
        wrap = jnp.concatenate([m0, new[0:R - NM]], axis=0) if CHAINS > 1 else m0
        jn = (n + 1) % T
        new = jnp.where(jn == 0, wrap, new)
        diff = pltpu.bitcast(new, i32) != pltpu.bitcast(mst[jn], i32)
        changed = jnp.max(diff.astype(i32))
        mst[jn] = new
        return n + 1, changed

    jax.lax.while_loop(
        lambda c: jnp.logical_and(c[0] < NSEG + T, jnp.logical_or(c[0] < T, c[1] > 0)),
        step, (jnp.int32(0), jnp.int32(1)))

    ng = NSEG // 4

    def out_copy(g):
        rows = pl.ds(pl.multiple_of(g * 128, 128), 128)
        return pltpu.make_async_copy(o_st.at[rows, :], o_hbm.at[rows, :], osem.at[g])

    def token_scores(g, a):
        rows = pl.ds(pl.multiple_of((4 * g + a) * SEG, SEG), SEG)
        ssc[g % 2, pl.ds(pl.multiple_of(SEG * a, SEG), SEG), :] = _dot(xs[rows, :], keys(4 * g + a))

    def tok(g, carry):
        kk = jax.lax.broadcasted_iota(i32, (SEG, 128), 0)
        tt = jax.lax.broadcasted_iota(i32, (SEG, 128), 1) % SEG
        st = ssc[g % 2].T
        for a in range(4):
            token_scores(jnp.minimum(g + 1, ng - 1), a)
        pt = _seg_softmax(st, kk <= tt).T
        for a in range(4):
            seg = 4 * g + a
            o = _dot(pt[SEG * a:SEG * (a + 1)].astype(bf16), values(seg))
            o_st[pl.ds(pl.multiple_of(seg * SEG, SEG), SEG), 0:DM] = _fold_rem(o).astype(bf16)
        out_copy(g).start()
        return carry

    jax.lax.fori_loop(0, 4, lambda a, c: token_scores(0, a), None)
    jax.lax.fori_loop(0, ng, tok, 0)
    for g in range(ng):
        out_copy(g).wait()


def _kernel(axt_hbm, m0_ref, awq_hbm, awk_hbm, awv_hbm, awot_hbm,
            bxt_hbm, bc_hbm, bwq_hbm, bwk_hbm, bwv_hbm, bwot_hbm, o_hbm,
            axt, axs, a3, b3, kt, acc, xsem):
    pl.run_scoped(
        functools.partial(_absorb, awq_hbm, awk_hbm, awv_hbm, awot_hbm,
                          pltpu.make_async_copy(axt_hbm, axt, xsem.at[0]), a3, b3),
        pltpu.VMEM((NP, DM, D), u32), pltpu.VMEM((NP, DM, D), u32), pltpu.VMEM((NP, DM, D), u32),
        pltpu.VMEM((NP, 2, DM, D), bf16), pltpu.SemaphoreType.DMA((4, NP)))
    pl.run_scoped(
        functools.partial(_branch_b, bxt_hbm, bc_hbm, bwq_hbm, bwk_hbm, bwv_hbm, bwot_hbm, acc,
                          functools.partial(_project_keys, axt, axs, a3, kt)),
        pltpu.VMEM((DM, S), bf16), pltpu.VMEM((S, DM), bf16), pltpu.VMEM((S, DC), bf16),
        pltpu.VMEM((2, DM, D), u32), pltpu.VMEM((2, DC, D), u32), pltpu.VMEM((2, DC, D), u32),
        pltpu.VMEM((2, 2, DM, D), bf16), pltpu.VMEM((2, DM, D), bf16), pltpu.VMEM((2, DC, 2 * D), bf16),
        pltpu.VMEM((S, D), bf16), pltpu.VMEM((S, D), bf16), pltpu.VMEM((S, D), bf16),
        pltpu.SemaphoreType.DMA((5, 2)))
    pl.run_scoped(
        functools.partial(_branch_a, m0_ref, o_hbm, acc, axs, a3, b3, kt),
        pltpu.VMEM((S, 2 * DM), bf16), pltpu.VMEM((NP, S, PW), bf16),
        pltpu.VMEM((NSEG, 128, 512), bf16), pltpu.VMEM((T, R, DM), f32), pltpu.VMEM((2, 128, NK), f32),
        pltpu.SemaphoreType.DMA((NSEG // 4,)))


@jax.jit
def pallas_concat_heads__memory_aug_recurrent_mem_tr__compressed_kv_cla__prompt_kernel(
    A_x, A_mem0, A_Wq, A_Wk, A_Wv, A_Wo, A_seg_len, B_x, B_c_kv, B_w_q, B_w_uk, B_w_uv, B_w_o,
):
    del A_seg_len
    assert A_x.shape == (1, S, DM) and B_c_kv.shape == (1, S, DC) and A_Wq.shape == (DM, H, D)
    hbm = lambda a: pltpu.with_memory_space_constraint(a, pltpu.HBM)
    in_hbm = pl.BlockSpec(memory_space=pltpu.HBM)
    out = pl.pallas_call(
        _kernel,
        out_shape=pltpu.HBM((S, 2 * DM), bf16),
        in_specs=[in_hbm, pl.BlockSpec(memory_space=pltpu.VMEM)] + [in_hbm] * 10,
        out_specs=in_hbm,
        scratch_shapes=[
            pltpu.VMEM((DM, S), bf16), pltpu.VMEM((S, DM), bf16), pltpu.VMEM((NP, PW, DM), bf16), pltpu.VMEM((NP, PW, DM), bf16),
            pltpu.VMEM((5, NSEG, DM, 128), bf16), pltpu.VMEM((DM, S), f32), pltpu.SemaphoreType.DMA((1,))],
        compiler_params=pltpu.CompilerParams(vmem_limit_bytes=120 * 1024 * 1024),
        name="fused_rmt_mla",
    )(hbm(A_x[0].T), A_mem0[0], hbm(A_Wq), hbm(A_Wk), hbm(A_Wv), hbm(A_Wo.transpose(0, 2, 1)),
      hbm(B_x[0].T), hbm(B_c_kv[0]), hbm(B_w_q), hbm(B_w_uk), hbm(B_w_uv), hbm(B_w_o.transpose(0, 2, 1)))
    return out[None]
```

```python
import functools
import math

import jax
import numpy as np
import jax.numpy as jnp
from jax.experimental import pallas as pl
from jax.experimental.pallas import tpu as pltpu

f32, bf16, u32, i32 = jnp.float32, jnp.bfloat16, jnp.uint32, jnp.int32
NT = (((1,), (1,)), ((), ()))

S, DM, DC, H, D = 2048, 448, 1024, 16, 256
NP = H // 2
NM, SEG = 8, 32
NSEG = S // SEG
MM = 384
PW = 2 * MM + 128
NK = H * (SEG + NM)
NEG = -1e30
LOG2E = math.log2(math.e)

CHAINS = 8
T = NSEG // CHAINS
R = NM * CHAINS
import os
BQ = int(os.environ.get('BQ', 256))
CK = 256
ORDER = os.environ.get('ORDER', 'Q0 p0 Q1 p1 Q2 p2 Q3 p3 s7 s6 a7 s5 a6 s4 a5 s3 a4 s2 o7 a3 s1 o6 a2 s0 o5 a1 o4 a0 o3 o2 o1 o0')
PRB = int(os.environ.get('PRB', 512))
PRA = 512
NKI = int(os.environ.get('NKI', 16))
NVI = int(os.environ.get('NVI', 16))


def _half(w, u):
    sh = np.uint32(16 * (1 - u)) if isinstance(u, int) else (16 * (1 - u)).astype(u32)
    return pltpu.bitcast((w << sh) & np.uint32(0xFFFF0000), f32).astype(bf16)


def _dot(a, b):
    return jnp.dot(a, b, preferred_element_type=f32)


def _dot_nt(a, b):
    return jax.lax.dot_general(a, b, NT, preferred_element_type=f32)


def _branch_b(xt_hbm, c_hbm, wq_hbm, wk_hbm, wv_hbm, wot_hbm, acc, overlapped_work,
              xt, xs, cs, wq_b, wk_b, wv_b, wo_b, wq1, wkv1, q_s, k_s, v_s, sems):
    wq32, wk32, wv32 = (r.bitcast(u32) for r in (wq_hbm, wk_hbm, wv_hbm))
    nsub, nq = BQ // 128, S // BQ

    def copies(p, slot):
        return [pltpu.make_async_copy(wq32.at[:, p, :], wq_b.at[slot], sems.at[0, slot]),
                pltpu.make_async_copy(wk32.at[:, p, :], wk_b.at[slot], sems.at[1, slot]),
                pltpu.make_async_copy(wv32.at[:, p, :], wv_b.at[slot], sems.at[2, slot]),
                pltpu.make_async_copy(wot_hbm.at[pl.ds(2 * p, 2)], wo_b.at[slot], sems.at[3, slot])]

    def prepare(h, r, n):
        slot, dst = (h // 2) % 2, h % 2
        half = lambda w: _half(w, h % 2)
        part = lambda w: pl.ds(r * w if isinstance(r, int) else pl.multiple_of(r * w, w), w)
        rq, rc = part(DM // n), part(DC // n)
        wq1[dst, rq, :] = half(wq_b[slot, rq, :])
        wkv1[dst, rc, 0:D] = half(wk_b[slot, rc, :])
        wkv1[dst, rc, D:2 * D] = half(wv_b[slot, rc, :])

    cx = pltpu.make_async_copy(xt_hbm, xt, sems.at[4, 0])
    cc = pltpu.make_async_copy(c_hbm, cs, sems.at[4, 1])
    for c in [cx, cc] + copies(0, 0) + copies(1, 1):
        c.start()
    overlapped_work()
    for c in [cx, cc] + copies(0, 0):
        c.wait()

    def first(r, carry):
        rows = pl.ds(pl.multiple_of(r * PRB, PRB), PRB)
        xs[rows, :] = xt[:, rows].T
        acc[:, rows] = jnp.zeros((DM, PRB), f32)
        prepare(0, r, S // PRB)
        return carry

    jax.lax.fori_loop(0, S // PRB, first, 0)
    qscale = (D ** -0.5) * LOG2E

    ri = jax.lax.broadcasted_iota(i32, (128, 128), 0)
    ci = jax.lax.broadcasted_iota(i32, (128, 128), 1)
    tri = ci <= ri

    def scores(i):
        r0 = i * BQ
        q = q_s[r0:r0 + BQ, :]
        chunks = [_dot_nt(q, k_s[c0:c0 + CK, :]) for c0 in range(0, r0, CK)]
        strips = []
        for a in range(nsub):
            t = _dot_nt(q[128 * a:, :], k_s[r0 + 128 * a:r0 + 128 * (a + 1), :])
            top = jnp.where(tri, t[0:128], NEG)
            strips.append(jnp.concatenate([top, t[128:]], axis=0) if a + 1 < nsub else top)
        return chunks, strips

    def attend(i, chunks, strips):
        r0 = i * BQ
        ms = []
        for b in range(nsub):
            parts = [t[128 * b:128 * (b + 1)] for t in chunks]
            parts += [strips[a][128 * (b - a):128 * (b - a + 1)] for a in range(b + 1)]
            ms.append(jnp.max(jnp.concatenate(parts, axis=1), axis=1, keepdims=True))
        m = jnp.concatenate(ms, axis=0)
        o = l = None
        for c, t in enumerate(chunks):
            e = jnp.exp2(t - m)
            for u in range(0, CK, 128):
                l = e[:, u:u + 128] if l is None else l + e[:, u:u + 128]
            pv = _dot(e.astype(bf16), v_s[c * CK:(c + 1) * CK, :])
            o = pv if o is None else o + pv
        os_ = [None if o is None else o[128 * b:128 * (b + 1)] for b in range(nsub)]
        ls = [None if l is None else l[128 * b:128 * (b + 1)] for b in range(nsub)]
        for a in range(nsub):
            e = jnp.exp2(strips[a] - m[128 * a:])
            pv = _dot(e.astype(bf16), v_s[r0 + 128 * a:r0 + 128 * (a + 1), :])
            for b in range(a, nsub):
                sl = slice(128 * (b - a), 128 * (b - a + 1))
                os_[b] = pv[sl] if os_[b] is None else os_[b] + pv[sl]
                ls[b] = e[sl] if ls[b] is None else ls[b] + e[sl]
        return jnp.concatenate(os_, axis=0), jnp.concatenate(ls, axis=0)

    def head(h, carry):
        p = h // 2

        @pl.when(jnp.logical_and(h % 2 == 1, h + 1 < H))
        def _():
            for c in copies(p + 1, (p + 1) % 2):
                c.wait()

        def project_in(r):
            rows = pl.ds(r * PRB, PRB)
            prepare(h + 1, r, S // PRB)
            kv = _dot(cs[rows, :], wkv1[h % 2]).astype(bf16)
            k_s[rows, :] = kv[:, 0:D]
            v_s[rows, :] = kv[:, D:2 * D]

        def project_out(i, o, l):
            ctx = (o * (1.0 / jnp.sum(l, axis=1, keepdims=True))).astype(bf16)
            acc[:, i * BQ:(i + 1) * BQ] += _dot_nt(wo_b[p % 2, h % 2], ctx)

        sc, ol = {}, {}
        for op in ORDER.split():
            i = int(op[1:])
            if op[0] == "p":
                project_in(i)
            elif op[0] in "qQ":
                n = BQ if op[0] == "q" else 2 * BQ
                rows = pl.ds(i * n, n)
                q_s[rows, :] = (_dot(xs[rows, :], wq1[h % 2]) * qscale).astype(bf16)
            elif op[0] == "s":
                sc[i] = scores(i)
            elif op[0] == "a":
                ol[i] = attend(i, *sc.pop(i))
            else:
                project_out(i, *ol.pop(i))

        @pl.when(jnp.logical_and(h % 2 == 1, p + 2 < NP))
        def _():
            for c in copies(p + 2, p % 2):
                c.start()

        return carry

    jax.lax.fori_loop(0, H, head, 0)


def _split_pair(z):
    rem = z[:, 2 * MM:]
    bits = rem if rem.dtype == f32 else pltpu.bitcast(rem, u32)
    low = jax.lax.broadcasted_iota(i32, bits.shape, 1) < 64
    zero = jnp.zeros_like(bits)
    r0, r1 = jnp.where(low, bits, zero), jnp.where(low, zero, bits)
    if rem.dtype != f32:
        r0, r1 = pltpu.bitcast(r0, rem.dtype), pltpu.bitcast(r1, rem.dtype)
    return (jnp.concatenate([z[:, 0:MM], r0], axis=1), jnp.concatenate([z[:, MM:2 * MM], r1], axis=1))


def _fold_rem(o):
    o3 = o[:, MM:]
    o3 = o3 + pltpu.roll(o3, 64, 1)
    return jnp.concatenate([o[:, 0:MM], o3[:, 0:DM - MM]], axis=1)


def _seg_softmax(st, mask):
    px, pm = [], []
    for h in range(H):
        sx = st[SEG * h:SEG * (h + 1), :]
        if mask is not None:
            sx = jnp.where(mask, sx, NEG)
        sm = st[H * SEG + NM * h:H * SEG + NM * (h + 1), :]
        m = jnp.maximum(jnp.max(sx, axis=0, keepdims=True), jnp.max(sm, axis=0, keepdims=True))
        ex = jnp.exp2(sx - m)
        em = jnp.exp2(sm - m)
        inv = 1.0 / (jnp.sum(ex, axis=0, keepdims=True) + jnp.sum(em, axis=0, keepdims=True))
        px.append(ex * inv)
        pm.append(em * inv)
    return jnp.concatenate(px + pm, axis=0)


def _chunk_transpose(t):
    lane = jax.lax.broadcasted_iota(i32, t[0].shape, 1)
    low = lane < 64
    even = (lane & 32) == 0
    u0 = jnp.where(low, t[0], pltpu.roll(t[2], 64, 1))
    u2 = jnp.where(low, pltpu.roll(t[0], 64, 1), t[2])
    u1 = jnp.where(low, t[1], pltpu.roll(t[3], 64, 1))
    u3 = jnp.where(low, pltpu.roll(t[1], 64, 1), t[3])
    return [jnp.where(even, u0, pltpu.roll(u1, 32, 1)), jnp.where(even, pltpu.roll(u0, 96, 1), u1),
            jnp.where(even, u2, pltpu.roll(u3, 32, 1)), jnp.where(even, pltpu.roll(u2, 96, 1), u3)]


def _absorb(wq_hbm, wk_hbm, wv_hbm, wot_hbm, xt_copy, a3, b3, wq_b, wk_b, wv_b, wo_b, sems):
    qscale = (D ** -0.5) * LOG2E
    w32 = [r.bitcast(u32) for r in (wq_hbm, wk_hbm, wv_hbm)]

    def copies(p):
        cs = [pltpu.make_async_copy(w32[j].at[:, p, :], b.at[p], sems.at[j, p])
              for j, b in enumerate((wq_b, wk_b, wv_b))]
        return cs + [pltpu.make_async_copy(wot_hbm.at[pl.ds(2 * p, 2)], wo_b.at[p], sems.at[3, p])]

    for c in copies(0) + copies(1):
        c.start()

    def pre(h, carry):
        p, u = h // 2, h % 2

        @pl.when(u == 0)
        def _():
            for c in copies(p):
                c.wait()

            @pl.when(p + 2 < NP)
            def _():
                for c in copies(p + 2):
                    c.start()

            @pl.when(p + 2 == NP)
            def _():
                xt_copy.start()

        q, k, v = (_half(b[p], u) for b in (wq_b, wk_b, wv_b))
        for dst, w in ((a3, _dot_nt(q, k) * qscale), (b3, _dot_nt(wo_b[p, u], v))):
            w = w.astype(bf16)
            dst[p, pl.ds(pl.multiple_of(u * MM, MM), MM), :] = w[0:MM]
            dst[p, pl.ds(pl.multiple_of(2 * MM + 64 * u, 64), 64), :] = w[MM:]
        return carry

    jax.lax.fori_loop(0, H, pre, 0)
    xt_copy.wait()


def _project_keys(xt, xs, a3, kt):
    per = NKI // (H // 4)
    nb = S // 128 // per
    nt = S // NKI

    def proj_k(i, carry):
        g, t0 = i // per, (i % per) * nb
        tok = pl.ds(pl.multiple_of(i * nt, nt), nt)
        xs[tok, :] = xt[:, tok].T
        starts = [(pp, u * MM + c if c < MM else 2 * MM + 64 * u)
                  for c in range(0, DM, 64) for pp in range(2) for u in range(2)]
        for tb in range(nb):
            xb = xt[:, pl.ds(pl.multiple_of((t0 + tb) * 128, 128), 128)]
            lhs = jnp.concatenate([a3[2 * g + pp, r0:r0 + 64, :] for pp, r0 in starts], axis=0)
            z = pltpu.bitcast(_dot(lhs, xb).astype(bf16), u32)
            for c in range(DM // 64):
                t = [z[32 * (4 * c + a):32 * (4 * c + a + 1)] for a in range(4)]
                for b, o in enumerate(_chunk_transpose(t)):
                    kt[g, 4 * (t0 + tb) + b, 64 * c:64 * (c + 1), :] = pltpu.bitcast(o, bf16)
        return carry

    jax.lax.fori_loop(0, NKI, proj_k, 0)


def _branch_a(m0_ref, o_hbm, acc, xs, a3, b3, kt, o_st, v3, vm, mst, ssc, psc, osem):
    def proj_v(i, carry):
        per, nt = NVI // NP, S // NVI
        p = i // per
        tok = pl.ds(pl.multiple_of(i * nt, nt), nt)
        o_st[tok, DM:2 * DM] = acc[:, tok].astype(bf16).T
        for r in range(S // PRA // per):
            rows = pl.ds(pl.multiple_of((i % per) * (S // per) + r * PRA, PRA), PRA)
            v3[p, rows, :] = _dot_nt(xs[rows, :], b3[p]).astype(bf16)
        return carry

    jax.lax.fori_loop(0, NVI, proj_v, 0)

    def block(i, n):
        return pl.ds(i * n if isinstance(i, int) else pl.multiple_of(i * n, n), n)

    def keys(seg):
        return jnp.concatenate([kt[g, seg] for g in range(5)], axis=1)

    def values(seg):
        rows = block(seg, SEG)
        hs = []
        for p in range(NP):
            hs += list(_split_pair(v3[p, rows, :]))
        return jnp.concatenate(hs + [vm[seg]], axis=0)

    m0 = m0_ref[...].astype(f32)
    mst[...] = jnp.zeros_like(mst)
    mst[0, 0:NM, :] = m0

    def step(carry):
        n, _ = carry
        j = n % T
        m = mst[j]
        mb = m.astype(bf16)
        zk = [_dot_nt(mb, a3[p]) for p in range(NP)]
        even = (jax.lax.broadcasted_iota(i32, (32, 128), 1) & NM) == 0
        for c in range(CHAINS):
            cr = slice(NM * c, NM * (c + 1))
            z = jnp.concatenate(
                [jnp.concatenate([zz[cr, u * MM:(u + 1) * MM], zz[cr, 2 * MM:]], axis=1)
                 for zz in zk for u in range(2)], axis=0).astype(bf16).T
            kt[4, c * T + j, 0:MM, :] = z[0:MM]
            kt[4, c * T + j, MM:, :] = pltpu.bitcast(
                jnp.where(even, pltpu.bitcast(z[MM:MM + 64], u32), pltpu.bitcast(z[MM + 64:], u32)), bf16)

        def mem_values(p):
            h0, h1 = _split_pair(_dot_nt(mb, b3[p]))
            for c in range(CHAINS):
                vm[c * T + j, 16 * p:16 * (p + 1), :] = jnp.concatenate(
                    [h0[NM * c:NM * (c + 1)], h1[NM * c:NM * (c + 1)]], axis=0).astype(bf16)

        for p in range(NP // 2):
            mem_values(p)
        ss = [_dot(m[NM * c:NM * (c + 1)].astype(bf16), keys(c * T + j)) for c in range(CHAINS)]
        if R < 128:
            ss.append(jnp.zeros((128 - R, NK), f32))
        for p in range(NP // 2, NP):
            mem_values(p)
        pt = _seg_softmax(jnp.concatenate(ss, axis=0).T, None).T
        os_ = [_dot(pt[NM * c:NM * (c + 1)].astype(bf16), values(c * T + j)) for c in range(CHAINS)]
        new = _fold_rem(jnp.concatenate(os_, axis=0)).astype(bf16).astype(f32)
        wrap = jnp.concatenate([m0, new[0:R - NM]], axis=0) if CHAINS > 1 else m0
        jn = (n + 1) % T
        new = jnp.where(jn == 0, wrap, new)
        diff = pltpu.bitcast(new, i32) != pltpu.bitcast(mst[jn], i32)
        changed = jnp.max(diff.astype(i32))
        mst[jn] = new
        return n + 1, changed

    jax.lax.while_loop(
        lambda c: jnp.logical_and(c[0] < NSEG + T, jnp.logical_or(c[0] < T, c[1] > 0)),
        step, (jnp.int32(0), jnp.int32(1)))

    ng = NSEG // 4

    def out_copy(g):
        return pltpu.make_async_copy(o_st.at[block(g, 128), :], o_hbm.at[block(g, 128), :], osem.at[g])

    ssc[...] = jnp.zeros_like(ssc)
    psc[...] = jnp.zeros_like(psc)

    def tok(i, carry):
        kk = jax.lax.broadcasted_iota(i32, (SEG, 128), 0)
        tt = jax.lax.broadcasted_iota(i32, (SEG, 128), 1) % SEG
        g2, g0 = jnp.maximum(i - 2, 0), jnp.minimum(i, ng - 1)
        p_old = psc[...]
        p_new = _seg_softmax(ssc[...].T, kk <= tt).T.astype(bf16)
        for a in range(4):
            o = _dot(p_old[SEG * a:SEG * (a + 1)], values(4 * g2 + a))
            o_st[block(4 * g2 + a, SEG), 0:DM] = _fold_rem(o).astype(bf16)
        for a in range(4):
            ssc[SEG * a:SEG * (a + 1), :] = _dot(xs[block(4 * g0 + a, SEG), :], keys(4 * g0 + a))
        psc[...] = p_new

        @pl.when(i >= 2)
        def _():
            out_copy(g2).start()

        return carry

    jax.lax.fori_loop(0, ng + 2, tok, 0)
    for g in range(ng):
        out_copy(g).wait()


def _kernel(axt_hbm, m0_ref, awq_hbm, awk_hbm, awv_hbm, awot_hbm,
            bxt_hbm, bc_hbm, bwq_hbm, bwk_hbm, bwv_hbm, bwot_hbm, o_hbm,
            axt, axs, a3, b3, kt, acc, xsem):
    pl.run_scoped(
        functools.partial(_absorb, awq_hbm, awk_hbm, awv_hbm, awot_hbm,
                          pltpu.make_async_copy(axt_hbm, axt, xsem.at[0]), a3, b3),
        pltpu.VMEM((NP, DM, D), u32), pltpu.VMEM((NP, DM, D), u32), pltpu.VMEM((NP, DM, D), u32),
        pltpu.VMEM((NP, 2, DM, D), bf16), pltpu.SemaphoreType.DMA((4, NP)))
    pl.run_scoped(
        functools.partial(_branch_b, bxt_hbm, bc_hbm, bwq_hbm, bwk_hbm, bwv_hbm, bwot_hbm, acc,
                          functools.partial(_project_keys, axt, axs, a3, kt)),
        pltpu.VMEM((DM, S), bf16), pltpu.VMEM((S, DM), bf16), pltpu.VMEM((S, DC), bf16),
        pltpu.VMEM((2, DM, D), u32), pltpu.VMEM((2, DC, D), u32), pltpu.VMEM((2, DC, D), u32),
        pltpu.VMEM((2, 2, DM, D), bf16), pltpu.VMEM((2, DM, D), bf16), pltpu.VMEM((2, DC, 2 * D), bf16),
        pltpu.VMEM((S, D), bf16), pltpu.VMEM((S, D), bf16), pltpu.VMEM((S, D), bf16),
        pltpu.SemaphoreType.DMA((5, 2)))
    pl.run_scoped(
        functools.partial(_branch_a, m0_ref, o_hbm, acc, axs, a3, b3, kt),
        pltpu.VMEM((S, 2 * DM), bf16), pltpu.VMEM((NP, S, PW), bf16),
        pltpu.VMEM((NSEG, 128, 512), bf16), pltpu.VMEM((T, R, DM), f32), pltpu.VMEM((128, NK), f32),
        pltpu.VMEM((128, NK), bf16),
        pltpu.SemaphoreType.DMA((NSEG // 4,)))


@jax.jit
def pallas_concat_heads__memory_aug_recurrent_mem_tr__compressed_kv_cla__prompt_kernel(
    A_x, A_mem0, A_Wq, A_Wk, A_Wv, A_Wo, A_seg_len, B_x, B_c_kv, B_w_q, B_w_uk, B_w_uv, B_w_o,
):
    del A_seg_len
    assert A_x.shape == (1, S, DM) and B_c_kv.shape == (1, S, DC) and A_Wq.shape == (DM, H, D)
    hbm = lambda a: pltpu.with_memory_space_constraint(a, pltpu.HBM)
    in_hbm = pl.BlockSpec(memory_space=pltpu.HBM)
    out = pl.pallas_call(
        _kernel,
        out_shape=pltpu.HBM((S, 2 * DM), bf16),
        in_specs=[in_hbm, pl.BlockSpec(memory_space=pltpu.VMEM)] + [in_hbm] * 10,
        out_specs=in_hbm,
        scratch_shapes=[
            pltpu.VMEM((DM, S), bf16), pltpu.VMEM((S, DM), bf16), pltpu.VMEM((NP, PW, DM), bf16), pltpu.VMEM((NP, PW, DM), bf16),
            pltpu.VMEM((5, NSEG, DM, 128), bf16), pltpu.VMEM((DM, S), f32), pltpu.SemaphoreType.DMA((1,))],
        compiler_params=pltpu.CompilerParams(vmem_limit_bytes=120 * 1024 * 1024),
        name="fused_rmt_mla",
    )(hbm(A_x[0].T), A_mem0[0], hbm(A_Wq), hbm(A_Wk), hbm(A_Wv), hbm(A_Wo.transpose(0, 2, 1)),
      hbm(B_x[0].T), hbm(B_c_kv[0]), hbm(B_w_q), hbm(B_w_uk), hbm(B_w_uv), hbm(B_w_o.transpose(0, 2, 1)))
    return out[None]
```

```python
import functools
import math

import jax
import numpy as np
import jax.numpy as jnp
from jax.experimental import pallas as pl
from jax.experimental.pallas import tpu as pltpu

f32, bf16, u32, i32 = jnp.float32, jnp.bfloat16, jnp.uint32, jnp.int32
NT = (((1,), (1,)), ((), ()))

S, DM, DC, H, D = 2048, 448, 1024, 16, 256
NP = H // 2
NM, SEG = 8, 32
NSEG = S // SEG
MM = 384
PW = 2 * MM + 128
NK = H * (SEG + NM)
NEG = -1e30
LOG2E = math.log2(math.e)

CHAINS = 8
T = NSEG // CHAINS
R = NM * CHAINS
import os
BQ = int(os.environ.get('BQ', 256))
CK = 256
AHEAD = int(os.environ.get('AHEAD', 2))
ORDER = os.environ.get('ORDER', 'Q0 p0 Q1 p1 Q2 p2 Q3 p3 s7 s6 a7 s5 a6 s4 a5 s3 a4 s2 o7 a3 s1 o6 a2 s0 o5 a1 o4 a0 o3 o2 o1 o0')
PRB = int(os.environ.get('PRB', 512))
PRA = 512
NKI = int(os.environ.get('NKI', 16))


def _half(w, u):
    sh = np.uint32(16 * (1 - u)) if isinstance(u, int) else (16 * (1 - u)).astype(u32)
    return pltpu.bitcast((w << sh) & np.uint32(0xFFFF0000), f32).astype(bf16)


def _dot(a, b):
    return jnp.dot(a, b, preferred_element_type=f32)


def _dot_nt(a, b):
    return jax.lax.dot_general(a, b, NT, preferred_element_type=f32)


def _branch_b(xt_hbm, c_hbm, wq_hbm, wk_hbm, wv_hbm, wot_hbm, acc, overlapped_work,
              xt, xs, cs, wq_b, wk_b, wv_b, wo_b, wq1, wkv1, q_s, k_s, v_s, sems):
    wq32, wk32, wv32 = (r.bitcast(u32) for r in (wq_hbm, wk_hbm, wv_hbm))
    nsub, nq = BQ // 128, S // BQ

    def copies(p, slot):
        return [pltpu.make_async_copy(wq32.at[:, p, :], wq_b.at[slot], sems.at[0, slot]),
                pltpu.make_async_copy(wk32.at[:, p, :], wk_b.at[slot], sems.at[1, slot]),
                pltpu.make_async_copy(wv32.at[:, p, :], wv_b.at[slot], sems.at[2, slot]),
                pltpu.make_async_copy(wot_hbm.at[pl.ds(2 * p, 2)], wo_b.at[slot], sems.at[3, slot])]

    def prepare(h, r, n):
        slot, dst = (h // 2) % 2, h % 2
        half = lambda w: _half(w, h % 2)
        part = lambda w: pl.ds(r * w if isinstance(r, int) else pl.multiple_of(r * w, w), w)
        rq, rc = part(DM // n), part(DC // n)
        wq1[dst, rq, :] = half(wq_b[slot, rq, :])
        wkv1[dst, rc, 0:D] = half(wk_b[slot, rc, :])
        wkv1[dst, rc, D:2 * D] = half(wv_b[slot, rc, :])

    cx = pltpu.make_async_copy(xt_hbm, xt, sems.at[4, 0])
    cc = pltpu.make_async_copy(c_hbm, cs, sems.at[4, 1])
    for c in [cx, cc] + copies(0, 0) + copies(1, 1):
        c.start()
    overlapped_work()
    for c in [cx, cc] + copies(0, 0):
        c.wait()

    def first(r, carry):
        rows = pl.ds(pl.multiple_of(r * PRB, PRB), PRB)
        xs[rows, :] = xt[:, rows].T
        acc[:, rows] = jnp.zeros((DM, PRB), f32)
        prepare(0, r, S // PRB)
        return carry

    jax.lax.fori_loop(0, S // PRB, first, 0)
    qscale = (D ** -0.5) * LOG2E

    ri = jax.lax.broadcasted_iota(i32, (128, 128), 0)
    ci = jax.lax.broadcasted_iota(i32, (128, 128), 1)
    tri = ci <= ri

    def scores(i):
        r0 = i * BQ
        q = q_s[r0:r0 + BQ, :]
        chunks = [_dot_nt(q, k_s[c0:c0 + CK, :]) for c0 in range(0, r0, CK)]
        strips = []
        for a in range(nsub):
            t = _dot_nt(q[128 * a:, :], k_s[r0 + 128 * a:r0 + 128 * (a + 1), :])
            top = jnp.where(tri, t[0:128], NEG)
            strips.append(jnp.concatenate([top, t[128:]], axis=0) if a + 1 < nsub else top)
        return chunks, strips

    def attend(i, chunks, strips):
        r0 = i * BQ
        ms = []
        for b in range(nsub):
            parts = [t[128 * b:128 * (b + 1)] for t in chunks]
            parts += [strips[a][128 * (b - a):128 * (b - a + 1)] for a in range(b + 1)]
            ms.append(jnp.max(jnp.concatenate(parts, axis=1), axis=1, keepdims=True))
        m = jnp.concatenate(ms, axis=0)
        o = l = None
        for c, t in enumerate(chunks):
            e = jnp.exp2(t - m)
            for u in range(0, CK, 128):
                l = e[:, u:u + 128] if l is None else l + e[:, u:u + 128]
            pv = _dot(e.astype(bf16), v_s[c * CK:(c + 1) * CK, :])
            o = pv if o is None else o + pv
        os_ = [None if o is None else o[128 * b:128 * (b + 1)] for b in range(nsub)]
        ls = [None if l is None else l[128 * b:128 * (b + 1)] for b in range(nsub)]
        for a in range(nsub):
            e = jnp.exp2(strips[a] - m[128 * a:])
            pv = _dot(e.astype(bf16), v_s[r0 + 128 * a:r0 + 128 * (a + 1), :])
            for b in range(a, nsub):
                sl = slice(128 * (b - a), 128 * (b - a + 1))
                os_[b] = pv[sl] if os_[b] is None else os_[b] + pv[sl]
                ls[b] = e[sl] if ls[b] is None else ls[b] + e[sl]
        return jnp.concatenate(os_, axis=0), jnp.concatenate(ls, axis=0)

    def head(h, carry):
        p = h // 2

        @pl.when(jnp.logical_and(h % 2 == 1, h + 1 < H))
        def _():
            for c in copies(p + 1, (p + 1) % 2):
                c.wait()

        def project_in(r):
            rows = pl.ds(r * PRB, PRB)
            prepare(h + 1, r, S // PRB)
            kv = _dot(cs[rows, :], wkv1[h % 2]).astype(bf16)
            k_s[rows, :] = kv[:, 0:D]
            v_s[rows, :] = kv[:, D:2 * D]

        def project_out(i, o, l):
            ctx = (o * (1.0 / jnp.sum(l, axis=1, keepdims=True))).astype(bf16)
            acc[:, i * BQ:(i + 1) * BQ] += _dot_nt(wo_b[p % 2, h % 2], ctx)

        sc, ol = {}, {}
        for op in ORDER.split():
            i = int(op[1:])
            if op[0] == "p":
                project_in(i)
            elif op[0] in "qQ":
                n = BQ if op[0] == "q" else 2 * BQ
                rows = pl.ds(i * n, n)
                q_s[rows, :] = (_dot(xs[rows, :], wq1[h % 2]) * qscale).astype(bf16)
            elif op[0] == "s":
                sc[i] = scores(i)
            elif op[0] == "a":
                ol[i] = attend(i, *sc.pop(i))
            else:
                project_out(i, *ol.pop(i))

        @pl.when(jnp.logical_and(h % 2 == 1, p + 2 < NP))
        def _():
            for c in copies(p + 2, p % 2):
                c.start()

        return carry

    jax.lax.fori_loop(0, H, head, 0)


def _split_pair(z):
    rem = z[:, 2 * MM:]
    bits = rem if rem.dtype == f32 else pltpu.bitcast(rem, u32)
    low = jax.lax.broadcasted_iota(i32, bits.shape, 1) < 64
    zero = jnp.zeros_like(bits)
    r0, r1 = jnp.where(low, bits, zero), jnp.where(low, zero, bits)
    if rem.dtype != f32:
        r0, r1 = pltpu.bitcast(r0, rem.dtype), pltpu.bitcast(r1, rem.dtype)
    return (jnp.concatenate([z[:, 0:MM], r0], axis=1), jnp.concatenate([z[:, MM:2 * MM], r1], axis=1))


def _fold_rem(o):
    o3 = o[:, MM:]
    o3 = o3 + pltpu.roll(o3, 64, 1)
    return jnp.concatenate([o[:, 0:MM], o3[:, 0:DM - MM]], axis=1)


def _seg_softmax(st, mask):
    px, pm = [], []
    for h in range(H):
        sx = st[SEG * h:SEG * (h + 1), :]
        if mask is not None:
            sx = jnp.where(mask, sx, NEG)
        sm = st[H * SEG + NM * h:H * SEG + NM * (h + 1), :]
        s = jnp.concatenate([sx, sm], axis=0)
        e = jnp.exp2(s - jnp.max(s, axis=0, keepdims=True))
        p = e * (1.0 / jnp.sum(e, axis=0, keepdims=True))
        px.append(p[0:SEG])
        pm.append(p[SEG:])
    return jnp.concatenate(px + pm, axis=0)


def _chunk_transpose(t):
    lane = jax.lax.broadcasted_iota(i32, t[0].shape, 1)
    low = lane < 64
    even = (lane & 32) == 0
    u0 = jnp.where(low, t[0], pltpu.roll(t[2], 64, 1))
    u2 = jnp.where(low, pltpu.roll(t[0], 64, 1), t[2])
    u1 = jnp.where(low, t[1], pltpu.roll(t[3], 64, 1))
    u3 = jnp.where(low, pltpu.roll(t[1], 64, 1), t[3])
    return [jnp.where(even, u0, pltpu.roll(u1, 32, 1)), jnp.where(even, pltpu.roll(u0, 96, 1), u1),
            jnp.where(even, u2, pltpu.roll(u3, 32, 1)), jnp.where(even, pltpu.roll(u2, 96, 1), u3)]


def _absorb(wq_hbm, wk_hbm, wv_hbm, wot_hbm, xt_copy, a3, b3, wq_b, wk_b, wv_b, wo_b, sems):
    qscale = (D ** -0.5) * LOG2E
    w32 = [r.bitcast(u32) for r in (wq_hbm, wk_hbm, wv_hbm)]

    def copies(p):
        cs = [pltpu.make_async_copy(w32[j].at[:, p, :], b.at[p], sems.at[j, p])
              for j, b in enumerate((wq_b, wk_b, wv_b))]
        return cs + [pltpu.make_async_copy(wot_hbm.at[pl.ds(2 * p, 2)], wo_b.at[p], sems.at[3, p])]

    for p in range(AHEAD):
        for c in copies(p):
            c.start()

    def pre(h, carry):
        p, u = h // 2, h % 2

        @pl.when(u == 0)
        def _():
            for c in copies(p):
                c.wait()

            @pl.when(p + AHEAD < NP)
            def _():
                for c in copies(p + AHEAD):
                    c.start()

            @pl.when(p + AHEAD == NP)
            def _():
                xt_copy.start()

        q, k, v = (_half(b[p], u) for b in (wq_b, wk_b, wv_b))
        for dst, w in ((a3, _dot_nt(q, k) * qscale), (b3, _dot_nt(wo_b[p, u], v))):
            w = w.astype(bf16)
            dst[p, pl.ds(pl.multiple_of(u * MM, MM), MM), :] = w[0:MM]
            dst[p, pl.ds(pl.multiple_of(2 * MM + 64 * u, 64), 64), :] = w[MM:]
        return carry

    jax.lax.fori_loop(0, H, pre, 0)
    xt_copy.wait()


def _project_tokens(xt, xs, a3, b3, kt, v3):
    per = NKI // (H // 4)
    nb = S // 128 // per

    def transpose(r, carry):
        tok = pl.ds(pl.multiple_of(r * PRA, PRA), PRA)
        xs[tok, :] = xt[:, tok].T
        return carry

    jax.lax.fori_loop(0, S // PRA, transpose, 0)

    def proj(i, carry):
        g, t0 = i // per, (i % per) * nb
        starts = [(pp, u * MM + c if c < MM else 2 * MM + 64 * u)
                  for c in range(0, DM, 64) for pp in range(2) for u in range(2)]
        for tb in range(nb):
            xb = xt[:, pl.ds(pl.multiple_of((t0 + tb) * 128, 128), 128)]
            lhs = jnp.concatenate([a3[2 * g + pp, r0:r0 + 64, :] for pp, r0 in starts], axis=0)
            z = pltpu.bitcast(_dot(lhs, xb).astype(bf16), u32)
            for c in range(DM // 64):
                t = [z[32 * (4 * c + a):32 * (4 * c + a + 1)] for a in range(4)]
                for b, o in enumerate(_chunk_transpose(t)):
                    kt[g, 4 * (t0 + tb) + b, 64 * c:64 * (c + 1), :] = pltpu.bitcast(o, bf16)
        rows = pl.ds(pl.multiple_of(t0 * 128, nb * 128), nb * 128)
        for pp in range(2):
            v3[2 * g + pp, rows, :] = _dot_nt(xs[rows, :], b3[2 * g + pp]).astype(bf16)
        return carry

    jax.lax.fori_loop(0, NKI, proj, 0)


def _branch_a(m0_ref, o_hbm, acc, xs, a3, b3, kt, v3, o_st, vm, mst, ssc, psc, osem):
    def block(i, n):
        return pl.ds(i * n if isinstance(i, int) else pl.multiple_of(i * n, n), n)

    def keys(seg):
        return jnp.concatenate([kt[g, seg] for g in range(5)], axis=1)

    def values(seg):
        rows = block(seg, SEG)
        hs = []
        for p in range(NP):
            hs += list(_split_pair(v3[p, rows, :]))
        return jnp.concatenate(hs + [vm[seg]], axis=0)

    m0 = m0_ref[...].astype(f32)
    mst[...] = jnp.zeros_like(mst)
    mst[0, 0:NM, :] = m0

    def step(carry):
        n, _ = carry
        j = n % T
        m = mst[j]
        mb = m.astype(bf16)
        zk = [_dot_nt(mb, a3[p]) for p in range(NP)]
        o_st[block(j, S // T), DM:2 * DM] = acc[:, block(j, S // T)].astype(bf16).T
        even = (jax.lax.broadcasted_iota(i32, (32, 128), 1) & NM) == 0
        for c in range(CHAINS):
            cr = slice(NM * c, NM * (c + 1))
            z = jnp.concatenate(
                [jnp.concatenate([zz[cr, u * MM:(u + 1) * MM], zz[cr, 2 * MM:]], axis=1)
                 for zz in zk for u in range(2)], axis=0).astype(bf16).T
            kt[4, c * T + j, 0:MM, :] = z[0:MM]
            kt[4, c * T + j, MM:, :] = pltpu.bitcast(
                jnp.where(even, pltpu.bitcast(z[MM:MM + 64], u32), pltpu.bitcast(z[MM + 64:], u32)), bf16)

        def mem_values(p):
            h0, h1 = _split_pair(_dot_nt(mb, b3[p]))
            for c in range(CHAINS):
                vm[c * T + j, 16 * p:16 * (p + 1), :] = jnp.concatenate(
                    [h0[NM * c:NM * (c + 1)], h1[NM * c:NM * (c + 1)]], axis=0).astype(bf16)

        for p in range(NP // 2):
            mem_values(p)
        ss = [_dot(m[NM * c:NM * (c + 1)].astype(bf16), keys(c * T + j)) for c in range(CHAINS)]
        if R < 128:
            ss.append(jnp.zeros((128 - R, NK), f32))
        for p in range(NP // 2, NP):
            mem_values(p)
        pt = _seg_softmax(jnp.concatenate(ss, axis=0).T, None).T
        os_ = [_dot(pt[NM * c:NM * (c + 1)].astype(bf16), values(c * T + j)) for c in range(CHAINS)]
        new = _fold_rem(jnp.concatenate(os_, axis=0)).astype(bf16).astype(f32)
        wrap = jnp.concatenate([m0, new[0:R - NM]], axis=0) if CHAINS > 1 else m0
        jn = (n + 1) % T
        new = jnp.where(jn == 0, wrap, new)
        diff = pltpu.bitcast(new, i32) != pltpu.bitcast(mst[jn], i32)
        changed = jnp.max(diff.astype(i32))
        mst[jn] = new
        return n + 1, changed

    jax.lax.while_loop(
        lambda c: jnp.logical_and(c[0] < NSEG + T, jnp.logical_or(c[0] < T, c[1] > 0)),
        step, (jnp.int32(0), jnp.int32(1)))

    ng = NSEG // 4

    def out_copy(g):
        return pltpu.make_async_copy(o_st.at[block(g, 128), :], o_hbm.at[block(g, 128), :], osem.at[g])

    ssc[...] = jnp.zeros_like(ssc)
    psc[...] = jnp.zeros_like(psc)

    def tok(i, carry):
        kk = jax.lax.broadcasted_iota(i32, (SEG, 128), 0)
        tt = jax.lax.broadcasted_iota(i32, (SEG, 128), 1) % SEG
        g2, g0 = jnp.maximum(i - 2, 0), jnp.minimum(i, ng - 1)
        p_old = psc[...]
        p_new = _seg_softmax(ssc[...].T, kk <= tt).T.astype(bf16)
        for a in range(4):
            o = _dot(p_old[SEG * a:SEG * (a + 1)], values(4 * g2 + a))
            o_st[block(4 * g2 + a, SEG), 0:DM] = _fold_rem(o).astype(bf16)
        for a in range(4):
            ssc[SEG * a:SEG * (a + 1), :] = _dot(xs[block(4 * g0 + a, SEG), :], keys(4 * g0 + a))
        psc[...] = p_new

        @pl.when(i >= 2)
        def _():
            out_copy(g2).start()

        return carry

    jax.lax.fori_loop(0, ng + 2, tok, 0)
    for g in range(ng):
        out_copy(g).wait()


def _kernel(axt_hbm, m0_ref, awq_hbm, awk_hbm, awv_hbm, awot_hbm,
            bxt_hbm, bc_hbm, bwq_hbm, bwk_hbm, bwv_hbm, bwot_hbm, o_hbm,
            axt, axs, a3, b3, kt, v3, acc, xsem):
    pl.run_scoped(
        functools.partial(_absorb, awq_hbm, awk_hbm, awv_hbm, awot_hbm,
                          pltpu.make_async_copy(axt_hbm, axt, xsem.at[0]), a3, b3),
        pltpu.VMEM((NP, DM, D), u32), pltpu.VMEM((NP, DM, D), u32), pltpu.VMEM((NP, DM, D), u32),
        pltpu.VMEM((NP, 2, DM, D), bf16), pltpu.SemaphoreType.DMA((4, NP)))
    pl.run_scoped(
        functools.partial(_branch_b, bxt_hbm, bc_hbm, bwq_hbm, bwk_hbm, bwv_hbm, bwot_hbm, acc,
                          functools.partial(_project_tokens, axt, axs, a3, b3, kt, v3)),
        pltpu.VMEM((DM, S), bf16), pltpu.VMEM((S, DM), bf16), pltpu.VMEM((S, DC), bf16),
        pltpu.VMEM((2, DM, D), u32), pltpu.VMEM((2, DC, D), u32), pltpu.VMEM((2, DC, D), u32),
        pltpu.VMEM((2, 2, DM, D), bf16), pltpu.VMEM((2, DM, D), bf16), pltpu.VMEM((2, DC, 2 * D), bf16),
        pltpu.VMEM((S, D), bf16), pltpu.VMEM((S, D), bf16), pltpu.VMEM((S, D), bf16),
        pltpu.SemaphoreType.DMA((5, 2)))
    pl.run_scoped(
        functools.partial(_branch_a, m0_ref, o_hbm, acc, axs, a3, b3, kt, v3),
        pltpu.VMEM((S, 2 * DM), bf16),
        pltpu.VMEM((NSEG, 128, 512), bf16), pltpu.VMEM((T, R, DM), f32), pltpu.VMEM((128, NK), f32),
        pltpu.VMEM((128, NK), bf16),
        pltpu.SemaphoreType.DMA((NSEG // 4,)))


@jax.jit
def pallas_concat_heads__memory_aug_recurrent_mem_tr__compressed_kv_cla__prompt_kernel(
    A_x, A_mem0, A_Wq, A_Wk, A_Wv, A_Wo, A_seg_len, B_x, B_c_kv, B_w_q, B_w_uk, B_w_uv, B_w_o,
):
    del A_seg_len
    assert A_x.shape == (1, S, DM) and B_c_kv.shape == (1, S, DC) and A_Wq.shape == (DM, H, D)
    in_hbm = pl.BlockSpec(memory_space=pltpu.HBM)
    out = pl.pallas_call(
        _kernel,
        out_shape=pltpu.HBM((S, 2 * DM), bf16),
        in_specs=[in_hbm, pl.BlockSpec(memory_space=pltpu.VMEM)] + [in_hbm] * 10,
        out_specs=in_hbm,
        scratch_shapes=[
            pltpu.VMEM((DM, S), bf16), pltpu.VMEM((S, DM), bf16), pltpu.VMEM((NP, PW, DM), bf16), pltpu.VMEM((NP, PW, DM), bf16),
            pltpu.VMEM((5, NSEG, DM, 128), bf16), pltpu.VMEM((NP, S, PW), bf16),
            pltpu.VMEM((DM, S), f32), pltpu.SemaphoreType.DMA((1,))],
        compiler_params=pltpu.CompilerParams(vmem_limit_bytes=120 * 1024 * 1024),
        name="fused_rmt_mla",
    )(A_x[0].T, A_mem0[0], A_Wq, A_Wk, A_Wv, A_Wo.transpose(0, 2, 1),
      B_x[0].T, B_c_kv[0], B_w_q, B_w_uk, B_w_uv, B_w_o.transpose(0, 2, 1))
    return out[None]
```

```python
import functools
import math

import jax
import numpy as np
import jax.numpy as jnp
from jax.experimental import pallas as pl
from jax.experimental.pallas import tpu as pltpu

f32, bf16, u32, i32 = jnp.float32, jnp.bfloat16, jnp.uint32, jnp.int32
NT = (((1,), (1,)), ((), ()))

S, DM, DC, H, D = 2048, 448, 1024, 16, 256
NP = H // 2
NM, SEG = 8, 32
NSEG = S // SEG
MM = 384
PW = 2 * MM + 128
NK = H * (SEG + NM)
NEG = -1e30
LOG2E = math.log2(math.e)

CHAINS = 8
T = NSEG // CHAINS
R = NM * CHAINS
import os
BQ = int(os.environ.get('BQ', 256))
CK = 256
ZV0 = int(os.environ.get('ZV0', 2))
ORDER = os.environ.get('ORDER', 'Q0 p0 Q1 p1 Q2 p2 Q3 p3 s7 s6 a7 s5 a6 s4 a5 s3 a4 s2 o7 a3 s1 o6 a2 s0 o5 a1 o4 a0 o3 o2 o1 o0')
PRB = int(os.environ.get('PRB', 512))
PRA = 512
NKI = int(os.environ.get('NKI', 16))


def _half(w, u):
    sh = np.uint32(16 * (1 - u)) if isinstance(u, int) else (16 * (1 - u)).astype(u32)
    return pltpu.bitcast((w << sh) & np.uint32(0xFFFF0000), f32).astype(bf16)


def _dot(a, b):
    return jnp.dot(a, b, preferred_element_type=f32)


def _dot_nt(a, b):
    return jax.lax.dot_general(a, b, NT, preferred_element_type=f32)


def _branch_b(xt_hbm, c_hbm, wq_hbm, wk_hbm, wv_hbm, wot_hbm, acc, overlapped_work,
              xt, xs, cs, wq_b, wk_b, wv_b, wo_b, wq1, wkv1, q_s, k_s, v_s, sems):
    wq32, wk32, wv32 = (r.bitcast(u32) for r in (wq_hbm, wk_hbm, wv_hbm))
    nsub, nq = BQ // 128, S // BQ

    def copies(p, slot):
        return [pltpu.make_async_copy(wq32.at[:, p, :], wq_b.at[slot], sems.at[0, slot]),
                pltpu.make_async_copy(wk32.at[:, p, :], wk_b.at[slot], sems.at[1, slot]),
                pltpu.make_async_copy(wv32.at[:, p, :], wv_b.at[slot], sems.at[2, slot]),
                pltpu.make_async_copy(wot_hbm.at[pl.ds(2 * p, 2)], wo_b.at[slot], sems.at[3, slot])]

    def prepare(h, r, n):
        slot, dst = (h // 2) % 2, h % 2
        half = lambda w: _half(w, h % 2)
        part = lambda w: pl.ds(r * w if isinstance(r, int) else pl.multiple_of(r * w, w), w)
        rq, rc = part(DM // n), part(DC // n)
        wq1[dst, rq, :] = half(wq_b[slot, rq, :])
        wkv1[dst, rc, 0:D] = half(wk_b[slot, rc, :])
        wkv1[dst, rc, D:2 * D] = half(wv_b[slot, rc, :])

    cx = pltpu.make_async_copy(xt_hbm, xt, sems.at[4, 0])
    cc = pltpu.make_async_copy(c_hbm, cs, sems.at[4, 1])
    for c in [cx, cc] + copies(0, 0) + copies(1, 1):
        c.start()
    overlapped_work()
    for c in [cx, cc] + copies(0, 0):
        c.wait()

    def first(r, carry):
        rows = pl.ds(pl.multiple_of(r * PRB, PRB), PRB)
        xs[rows, :] = xt[:, rows].T
        acc[:, rows] = jnp.zeros((DM, PRB), f32)
        prepare(0, r, S // PRB)
        return carry

    jax.lax.fori_loop(0, S // PRB, first, 0)
    qscale = (D ** -0.5) * LOG2E

    ri = jax.lax.broadcasted_iota(i32, (128, 128), 0)
    ci = jax.lax.broadcasted_iota(i32, (128, 128), 1)
    tri = ci <= ri

    def scores(i):
        r0 = i * BQ
        q = q_s[r0:r0 + BQ, :]
        chunks = [_dot_nt(q, k_s[c0:c0 + CK, :]) for c0 in range(0, r0, CK)]
        strips = []
        for a in range(nsub):
            t = _dot_nt(q[128 * a:, :], k_s[r0 + 128 * a:r0 + 128 * (a + 1), :])
            top = jnp.where(tri, t[0:128], NEG)
            strips.append(jnp.concatenate([top, t[128:]], axis=0) if a + 1 < nsub else top)
        return chunks, strips

    def attend(i, chunks, strips):
        r0 = i * BQ
        ms = []
        for b in range(nsub):
            parts = [t[128 * b:128 * (b + 1)] for t in chunks]
            parts += [strips[a][128 * (b - a):128 * (b - a + 1)] for a in range(b + 1)]
            ms.append(jnp.max(jnp.concatenate(parts, axis=1), axis=1, keepdims=True))
        m = jnp.concatenate(ms, axis=0)
        o = l = None
        for c, t in enumerate(chunks):
            e = jnp.exp2(t - m)
            for u in range(0, CK, 128):
                l = e[:, u:u + 128] if l is None else l + e[:, u:u + 128]
            pv = _dot(e.astype(bf16), v_s[c * CK:(c + 1) * CK, :])
            o = pv if o is None else o + pv
        os_ = [None if o is None else o[128 * b:128 * (b + 1)] for b in range(nsub)]
        ls = [None if l is None else l[128 * b:128 * (b + 1)] for b in range(nsub)]
        for a in range(nsub):
            e = jnp.exp2(strips[a] - m[128 * a:])
            pv = _dot(e.astype(bf16), v_s[r0 + 128 * a:r0 + 128 * (a + 1), :])
            for b in range(a, nsub):
                sl = slice(128 * (b - a), 128 * (b - a + 1))
                os_[b] = pv[sl] if os_[b] is None else os_[b] + pv[sl]
                ls[b] = e[sl] if ls[b] is None else ls[b] + e[sl]
        return jnp.concatenate(os_, axis=0), jnp.concatenate(ls, axis=0)

    def head(h, carry):
        p = h // 2

        @pl.when(jnp.logical_and(h % 2 == 1, h + 1 < H))
        def _():
            for c in copies(p + 1, (p + 1) % 2):
                c.wait()

        def project_in(r):
            rows = pl.ds(r * PRB, PRB)
            prepare(h + 1, r, S // PRB)
            kv = _dot(cs[rows, :], wkv1[h % 2]).astype(bf16)
            k_s[rows, :] = kv[:, 0:D]
            v_s[rows, :] = kv[:, D:2 * D]

        def project_out(i, o, l):
            ctx = (o * (1.0 / jnp.sum(l, axis=1, keepdims=True))).astype(bf16)
            acc[:, i * BQ:(i + 1) * BQ] += _dot_nt(wo_b[p % 2, h % 2], ctx)

        sc, ol = {}, {}
        for op in ORDER.split():
            i = int(op[1:])
            if op[0] == "p":
                project_in(i)
            elif op[0] in "qQ":
                n = BQ if op[0] == "q" else 2 * BQ
                rows = pl.ds(i * n, n)
                q_s[rows, :] = (_dot(xs[rows, :], wq1[h % 2]) * qscale).astype(bf16)
            elif op[0] == "s":
                sc[i] = scores(i)
            elif op[0] == "a":
                ol[i] = attend(i, *sc.pop(i))
            else:
                project_out(i, *ol.pop(i))

        @pl.when(jnp.logical_and(h % 2 == 1, p + 2 < NP))
        def _():
            for c in copies(p + 2, p % 2):
                c.start()

        return carry

    jax.lax.fori_loop(0, H, head, 0)


def _split_pair(z):
    rem = z[:, 2 * MM:]
    bits = rem if rem.dtype == f32 else pltpu.bitcast(rem, u32)
    low = jax.lax.broadcasted_iota(i32, bits.shape, 1) < 64
    zero = jnp.zeros_like(bits)
    r0, r1 = jnp.where(low, bits, zero), jnp.where(low, zero, bits)
    if rem.dtype != f32:
        r0, r1 = pltpu.bitcast(r0, rem.dtype), pltpu.bitcast(r1, rem.dtype)
    return (jnp.concatenate([z[:, 0:MM], r0], axis=1), jnp.concatenate([z[:, MM:2 * MM], r1], axis=1))


def _fold_rem(o):
    o3 = o[:, MM:]
    o3 = o3 + pltpu.roll(o3, 64, 1)
    return jnp.concatenate([o[:, 0:MM], o3[:, 0:DM - MM]], axis=1)


def _seg_softmax(st, mask):
    px, pm = [], []
    for h in range(H):
        sx = st[SEG * h:SEG * (h + 1), :]
        if mask is not None:
            sx = jnp.where(mask, sx, NEG)
        sm = st[H * SEG + NM * h:H * SEG + NM * (h + 1), :]
        s = jnp.concatenate([sx, sm], axis=0)
        e = jnp.exp2(s - jnp.max(s, axis=0, keepdims=True))
        p = e * (1.0 / jnp.sum(e, axis=0, keepdims=True))
        px.append(p[0:SEG])
        pm.append(p[SEG:])
    return jnp.concatenate(px + pm, axis=0)


def _chunk_transpose(t):
    lane = jax.lax.broadcasted_iota(i32, t[0].shape, 1)
    low = lane < 64
    even = (lane & 32) == 0
    u0 = jnp.where(low, t[0], pltpu.roll(t[2], 64, 1))
    u2 = jnp.where(low, pltpu.roll(t[0], 64, 1), t[2])
    u1 = jnp.where(low, t[1], pltpu.roll(t[3], 64, 1))
    u3 = jnp.where(low, pltpu.roll(t[1], 64, 1), t[3])
    return [jnp.where(even, u0, pltpu.roll(u1, 32, 1)), jnp.where(even, pltpu.roll(u0, 96, 1), u1),
            jnp.where(even, u2, pltpu.roll(u3, 32, 1)), jnp.where(even, pltpu.roll(u2, 96, 1), u3)]


def _absorb(wq_hbm, wk_hbm, wv_hbm, wot_hbm, xt_copy, a3, b3, wq_b, wk_b, wv_b, wo_b, sems):
    qscale = (D ** -0.5) * LOG2E
    w32 = [r.bitcast(u32) for r in (wq_hbm, wk_hbm, wv_hbm)]

    def copies(p):
        cs = [pltpu.make_async_copy(w32[j].at[:, p, :], b.at[p], sems.at[j, p])
              for j, b in enumerate((wq_b, wk_b, wv_b))]
        return cs + [pltpu.make_async_copy(wot_hbm.at[pl.ds(2 * p, 2)], wo_b.at[p], sems.at[3, p])]

    for c in copies(0):
        c.start()

    def pre(h, carry):
        p, u = h // 2, h % 2

        @pl.when(u == 0)
        def _():
            for c in copies(p):
                c.wait()

            @pl.when(p == 0)
            def _():
                for c in copies(1):
                    c.start()

            @pl.when(p + 2 < NP)
            def _():
                for c in copies(p + 2):
                    c.start()

            @pl.when(p + 2 == NP)
            def _():
                xt_copy.start()

        q, k, v = (_half(b[p], u) for b in (wq_b, wk_b, wv_b))
        for dst, w in ((a3, _dot_nt(q, k) * qscale), (b3, _dot_nt(wo_b[p, u], v))):
            w = w.astype(bf16)
            dst[p, pl.ds(pl.multiple_of(u * MM, MM), MM), :] = w[0:MM]
            dst[p, pl.ds(pl.multiple_of(2 * MM + 64 * u, 64), 64), :] = w[MM:]
        return carry

    jax.lax.fori_loop(0, H, pre, 0)
    xt_copy.wait()


def _project_tokens(xt, xs, a3, b3, kt, v3):
    per = NKI // (H // 4)
    nb = S // 128 // per

    def proj(i, carry):
        g, t0 = i // per, (i % per) * nb
        rows = pl.ds(pl.multiple_of(t0 * 128, nb * 128), nb * 128)
        xs[rows, :] = xt[:, rows].T
        starts = [(pp, u * MM + c if c < MM else 2 * MM + 64 * u)
                  for c in range(0, DM, 64) for pp in range(2) for u in range(2)]
        for tb in range(nb):
            xb = xt[:, pl.ds(pl.multiple_of((t0 + tb) * 128, 128), 128)]
            lhs = jnp.concatenate([a3[2 * g + pp, r0:r0 + 64, :] for pp, r0 in starts], axis=0)
            z = pltpu.bitcast(_dot(lhs, xb).astype(bf16), u32)
            for c in range(DM // 64):
                t = [z[32 * (4 * c + a):32 * (4 * c + a + 1)] for a in range(4)]
                for b, o in enumerate(_chunk_transpose(t)):
                    kt[g, 4 * (t0 + tb) + b, 64 * c:64 * (c + 1), :] = pltpu.bitcast(o, bf16)
        for pp in range(2):
            v3[2 * g + pp, rows, :] = _dot_nt(xs[rows, :], b3[2 * g + pp]).astype(bf16)
        return carry

    jax.lax.fori_loop(0, NKI, proj, 0)


def _branch_a(m0_ref, o_hbm, acc, xs, a3, b3, kt, v3, o_st, vm, mst, osem):
    def block(i, n):
        return pl.ds(i * n if isinstance(i, int) else pl.multiple_of(i * n, n), n)

    def keys(seg):
        return jnp.concatenate([kt[g, seg] for g in range(5)], axis=1)

    def values(seg):
        rows = block(seg, SEG)
        hs = []
        for p in range(NP):
            hs += list(_split_pair(v3[p, rows, :]))
        return jnp.concatenate(hs + [vm[seg]], axis=0)

    m0 = m0_ref[...].astype(f32)
    mst[...] = jnp.zeros_like(mst)
    mst[0, 0:NM, :] = m0

    def out_copies(j):
        rows = [block(c * T + j, SEG) for c in range(CHAINS)]
        return [pltpu.make_async_copy(o_st.at[r, :], o_hbm.at[r, :], osem.at[j]) for r in rows]

    def step(carry):
        n, _ = carry
        j = n % T

        @pl.when(n >= T)
        def _():
            for c in out_copies(j):
                c.wait()

        m = mst[j]
        mb = m.astype(bf16)
        zk = [_dot_nt(mb, a3[p]) for p in range(NP)]
        o_st[block(jnp.minimum(n, T), S // T), DM:2 * DM] = acc[:, block(j, S // T)].astype(bf16).T
        even = (jax.lax.broadcasted_iota(i32, (32, 128), 1) & NM) == 0
        for c in range(CHAINS):
            cr = slice(NM * c, NM * (c + 1))
            z = jnp.concatenate(
                [jnp.concatenate([zz[cr, u * MM:(u + 1) * MM], zz[cr, 2 * MM:]], axis=1)
                 for zz in zk for u in range(2)], axis=0).astype(bf16).T
            kt[4, c * T + j, 0:MM, :] = z[0:MM]
            kt[4, c * T + j, MM:, :] = pltpu.bitcast(
                jnp.where(even, pltpu.bitcast(z[MM:MM + 64], u32), pltpu.bitcast(z[MM + 64:], u32)), bf16)

        def mem_values(p):
            h0, h1 = _split_pair(_dot_nt(mb, b3[p]))
            for c in range(CHAINS):
                vm[c * T + j, 16 * p:16 * (p + 1), :] = jnp.concatenate(
                    [h0[NM * c:NM * (c + 1)], h1[NM * c:NM * (c + 1)]], axis=0).astype(bf16)

        for p in range(ZV0):
            mem_values(p)
        ss = [_dot(jnp.concatenate([xs[block(c * T + j, SEG), :], m[NM * c:NM * (c + 1)].astype(bf16)], axis=0),
                   keys(c * T + j)) for c in range(CHAINS)]
        for p in range(ZV0, NP):
            mem_values(p)
        kk = jax.lax.broadcasted_iota(i32, (SEG, 128), 0)
        tt = jax.lax.broadcasted_iota(i32, (SEG, 128), 1) % SEG
        sm = [t[SEG:] for t in ss] + ([jnp.zeros((128 - R, NK), f32)] if R < 128 else [])
        pm = _seg_softmax(jnp.concatenate(sm, axis=0).T, None).T
        px = [_seg_softmax(jnp.concatenate([t[0:SEG] for t in ss[c:c + 4]], axis=0).T, kk <= tt).T
              for c in range(0, CHAINS, 4)]
        os_ = []
        for c in range(CHAINS):
            pc = jnp.concatenate([px[c // 4][SEG * (c % 4):SEG * (c % 4 + 1)], pm[NM * c:NM * (c + 1)]], axis=0)
            o = _fold_rem(_dot(pc.astype(bf16), values(c * T + j)))
            o_st[block(c * T + j, SEG), 0:DM] = o[0:SEG].astype(bf16)
            os_.append(o[SEG:])
        new = jnp.concatenate(os_, axis=0).astype(bf16).astype(f32)
        wrap = jnp.concatenate([m0, new[0:R - NM]], axis=0) if CHAINS > 1 else m0
        jn = (n + 1) % T
        new = jnp.where(jn == 0, wrap, new)
        diff = pltpu.bitcast(new, i32) != pltpu.bitcast(mst[jn], i32)
        changed = jnp.max(diff.astype(i32))
        mst[jn] = new

        @pl.when(n >= T - 1)
        def _():
            def send(jj, carry):
                for c in out_copies(jj):
                    c.start()
                return carry

            jax.lax.fori_loop(jnp.where(n == T - 1, 0, j), j + 1, send, 0)

        return n + 1, changed

    jax.lax.while_loop(
        lambda c: jnp.logical_and(c[0] < NSEG + T, jnp.logical_or(c[0] < T, c[1] > 0)),
        step, (jnp.int32(0), jnp.int32(1)))


    def drain(j, carry):
        for c in out_copies(j):
            c.wait()
        return carry

    jax.lax.fori_loop(0, T, drain, 0)


def _kernel(axt_hbm, m0_ref, awq_hbm, awk_hbm, awv_hbm, awot_hbm,
            bxt_hbm, bc_hbm, bwq_hbm, bwk_hbm, bwv_hbm, bwot_hbm, o_hbm,
            axt, axs, a3, b3, kt, v3, acc, xsem):
    pl.run_scoped(
        functools.partial(_absorb, awq_hbm, awk_hbm, awv_hbm, awot_hbm,
                          pltpu.make_async_copy(axt_hbm, axt, xsem.at[0]), a3, b3),
        pltpu.VMEM((NP, DM, D), u32), pltpu.VMEM((NP, DM, D), u32), pltpu.VMEM((NP, DM, D), u32),
        pltpu.VMEM((NP, 2, DM, D), bf16), pltpu.SemaphoreType.DMA((4, NP)))
    pl.run_scoped(
        functools.partial(_branch_b, bxt_hbm, bc_hbm, bwq_hbm, bwk_hbm, bwv_hbm, bwot_hbm, acc,
                          functools.partial(_project_tokens, axt, axs, a3, b3, kt, v3)),
        pltpu.VMEM((DM, S), bf16), pltpu.VMEM((S, DM), bf16), pltpu.VMEM((S, DC), bf16),
        pltpu.VMEM((2, DM, D), u32), pltpu.VMEM((2, DC, D), u32), pltpu.VMEM((2, DC, D), u32),
        pltpu.VMEM((2, 2, DM, D), bf16), pltpu.VMEM((2, DM, D), bf16), pltpu.VMEM((2, DC, 2 * D), bf16),
        pltpu.VMEM((S, D), bf16), pltpu.VMEM((S, D), bf16), pltpu.VMEM((S, D), bf16),
        pltpu.SemaphoreType.DMA((5, 2)))
    pl.run_scoped(
        functools.partial(_branch_a, m0_ref, o_hbm, acc, axs, a3, b3, kt, v3),
        pltpu.VMEM((S + S // T, 2 * DM), bf16),
        pltpu.VMEM((NSEG, 128, 512), bf16), pltpu.VMEM((T, R, DM), f32),
        pltpu.SemaphoreType.DMA((T,)))


@jax.jit
def pallas_concat_heads__memory_aug_recurrent_mem_tr__compressed_kv_cla__prompt_kernel(
    A_x, A_mem0, A_Wq, A_Wk, A_Wv, A_Wo, A_seg_len, B_x, B_c_kv, B_w_q, B_w_uk, B_w_uv, B_w_o,
):
    del A_seg_len
    assert A_x.shape == (1, S, DM) and B_c_kv.shape == (1, S, DC) and A_Wq.shape == (DM, H, D)
    in_hbm = pl.BlockSpec(memory_space=pltpu.HBM)
    out = pl.pallas_call(
        _kernel,
        out_shape=pltpu.HBM((S, 2 * DM), bf16),
        in_specs=[in_hbm, pl.BlockSpec(memory_space=pltpu.VMEM)] + [in_hbm] * 10,
        out_specs=in_hbm,
        scratch_shapes=[
            pltpu.VMEM((DM, S), bf16), pltpu.VMEM((S, DM), bf16), pltpu.VMEM((NP, PW, DM), bf16), pltpu.VMEM((NP, PW, DM), bf16),
            pltpu.VMEM((5, NSEG, DM, 128), bf16), pltpu.VMEM((NP, S, PW), bf16),
            pltpu.VMEM((DM, S), f32), pltpu.SemaphoreType.DMA((1,))],
        compiler_params=pltpu.CompilerParams(vmem_limit_bytes=120 * 1024 * 1024),
        name="fused_rmt_mla",
    )(A_x[0].T, A_mem0[0], A_Wq, A_Wk, A_Wv, A_Wo.transpose(0, 2, 1),
      B_x[0].T, B_c_kv[0], B_w_q, B_w_uk, B_w_uv, B_w_o.transpose(0, 2, 1))
    return out[None]
```

```python
import functools
import math

import jax
import numpy as np
import jax.numpy as jnp
from jax.experimental import pallas as pl
from jax.experimental.pallas import tpu as pltpu

f32, bf16, u32, i32 = jnp.float32, jnp.bfloat16, jnp.uint32, jnp.int32
NT = (((1,), (1,)), ((), ()))

S, DM, DC, H, D = 2048, 448, 1024, 16, 256
NP = H // 2
NM, SEG = 8, 32
NSEG = S // SEG
MM = 384
PW = 2 * MM + 128
NK = H * (SEG + NM)
NEG = -1e30
LOG2E = math.log2(math.e)

CHAINS = 8
T = NSEG // CHAINS
R = NM * CHAINS
assert CHAINS == T
BQ = 256
CK = 256
ZV0 = 2
ORDER = ("Q0 p0 Q1 p1 Q2 p2 Q3 p3 s7 s6 a7 s5 a6 s4 a5 s3 a4 s2 o7 a3"
         " s1 o6 a2 s0 o5 a1 o4 a0 o3 o2 o1 o0")
PRB = 512
NKI = 16


def _half(w, u):
    sh = np.uint32(16 * (1 - u)) if isinstance(u, int) else (16 * (1 - u)).astype(u32)
    return pltpu.bitcast((w << sh) & np.uint32(0xFFFF0000), f32).astype(bf16)


def _dot(a, b):
    return jnp.dot(a, b, preferred_element_type=f32)


def _dot_nt(a, b):
    return jax.lax.dot_general(a, b, NT, preferred_element_type=f32)


def _branch_b(xt_hbm, c_hbm, wq_hbm, wk_hbm, wv_hbm, wot_hbm, acc, overlapped_work,
              xt, xs, cs, wq_b, wk_b, wv_b, wo_b, wq1, wkv1, q_s, k_s, v_s, sems):
    wq32, wk32, wv32 = (r.bitcast(u32) for r in (wq_hbm, wk_hbm, wv_hbm))
    nsub, nq = BQ // 128, S // BQ

    def copies(p, slot):
        return [pltpu.make_async_copy(wq32.at[:, p, :], wq_b.at[slot], sems.at[0, slot]),
                pltpu.make_async_copy(wk32.at[:, p, :], wk_b.at[slot], sems.at[1, slot]),
                pltpu.make_async_copy(wv32.at[:, p, :], wv_b.at[slot], sems.at[2, slot]),
                pltpu.make_async_copy(wot_hbm.at[pl.ds(2 * p, 2)], wo_b.at[slot], sems.at[3, slot])]

    def prepare(h, r, n):
        slot, dst = (h // 2) % 2, h % 2
        half = lambda w: _half(w, h % 2)
        part = lambda w: pl.ds(r * w if isinstance(r, int) else pl.multiple_of(r * w, w), w)
        rq, rc = part(DM // n), part(DC // n)
        wq1[dst, rq, :] = half(wq_b[slot, rq, :])
        wkv1[dst, rc, 0:D] = half(wk_b[slot, rc, :])
        wkv1[dst, rc, D:2 * D] = half(wv_b[slot, rc, :])

    cx = pltpu.make_async_copy(xt_hbm, xt, sems.at[4, 0])
    cc = pltpu.make_async_copy(c_hbm, cs, sems.at[4, 1])
    for c in [cx, cc] + copies(0, 0) + copies(1, 1):
        c.start()
    overlapped_work()
    for c in [cx, cc] + copies(0, 0):
        c.wait()

    def first(r, carry):
        rows = pl.ds(pl.multiple_of(r * PRB, PRB), PRB)
        xs[rows, :] = xt[:, rows].T
        acc[:, rows] = jnp.zeros((DM, PRB), f32)
        prepare(0, r, S // PRB)
        return carry

    jax.lax.fori_loop(0, S // PRB, first, 0)
    qscale = (D ** -0.5) * LOG2E

    ri = jax.lax.broadcasted_iota(i32, (128, 128), 0)
    ci = jax.lax.broadcasted_iota(i32, (128, 128), 1)
    tri = ci <= ri

    def scores(i):
        r0 = i * BQ
        q = q_s[r0:r0 + BQ, :]
        chunks = [_dot_nt(q, k_s[c0:c0 + CK, :]) for c0 in range(0, r0, CK)]
        strips = []
        for a in range(nsub):
            t = _dot_nt(q[128 * a:, :], k_s[r0 + 128 * a:r0 + 128 * (a + 1), :])
            top = jnp.where(tri, t[0:128], NEG)
            strips.append(jnp.concatenate([top, t[128:]], axis=0) if a + 1 < nsub else top)
        return chunks, strips

    def attend(i, chunks, strips):
        r0 = i * BQ
        ms = []
        for b in range(nsub):
            parts = [t[128 * b:128 * (b + 1)] for t in chunks]
            parts += [strips[a][128 * (b - a):128 * (b - a + 1)] for a in range(b + 1)]
            ms.append(jnp.max(jnp.concatenate(parts, axis=1), axis=1, keepdims=True))
        m = jnp.concatenate(ms, axis=0)
        o = l = None
        for c, t in enumerate(chunks):
            e = jnp.exp2(t - m)
            for u in range(0, CK, 128):
                l = e[:, u:u + 128] if l is None else l + e[:, u:u + 128]
            pv = _dot(e.astype(bf16), v_s[c * CK:(c + 1) * CK, :])
            o = pv if o is None else o + pv
        os_ = [None if o is None else o[128 * b:128 * (b + 1)] for b in range(nsub)]
        ls = [None if l is None else l[128 * b:128 * (b + 1)] for b in range(nsub)]
        for a in range(nsub):
            e = jnp.exp2(strips[a] - m[128 * a:])
            pv = _dot(e.astype(bf16), v_s[r0 + 128 * a:r0 + 128 * (a + 1), :])
            for b in range(a, nsub):
                sl = slice(128 * (b - a), 128 * (b - a + 1))
                os_[b] = pv[sl] if os_[b] is None else os_[b] + pv[sl]
                ls[b] = e[sl] if ls[b] is None else ls[b] + e[sl]
        return jnp.concatenate(os_, axis=0), jnp.concatenate(ls, axis=0)

    def head(h, carry):
        p = h // 2

        @pl.when(jnp.logical_and(h % 2 == 1, h + 1 < H))
        def _():
            for c in copies(p + 1, (p + 1) % 2):
                c.wait()

        def project_in(r):
            rows = pl.ds(r * PRB, PRB)
            prepare(h + 1, r, S // PRB)
            kv = _dot(cs[rows, :], wkv1[h % 2]).astype(bf16)
            k_s[rows, :] = kv[:, 0:D]
            v_s[rows, :] = kv[:, D:2 * D]

        def project_out(i, o, l):
            ctx = (o * (1.0 / jnp.sum(l, axis=1, keepdims=True))).astype(bf16)
            acc[:, i * BQ:(i + 1) * BQ] += _dot_nt(wo_b[p % 2, h % 2], ctx)

        sc, ol = {}, {}
        for op in ORDER.split():
            i = int(op[1:])
            if op[0] == "p":
                project_in(i)
            elif op[0] in "qQ":
                n = BQ if op[0] == "q" else 2 * BQ
                rows = pl.ds(i * n, n)
                q_s[rows, :] = (_dot(xs[rows, :], wq1[h % 2]) * qscale).astype(bf16)
            elif op[0] == "s":
                sc[i] = scores(i)
            elif op[0] == "a":
                ol[i] = attend(i, *sc.pop(i))
            else:
                project_out(i, *ol.pop(i))

        @pl.when(jnp.logical_and(h % 2 == 1, p + 2 < NP))
        def _():
            for c in copies(p + 2, p % 2):
                c.start()

        return carry

    jax.lax.fori_loop(0, H, head, 0)


def _split_pair(z):
    rem = z[:, 2 * MM:]
    bits = rem if rem.dtype == f32 else pltpu.bitcast(rem, u32)
    low = jax.lax.broadcasted_iota(i32, bits.shape, 1) < 64
    zero = jnp.zeros_like(bits)
    r0, r1 = jnp.where(low, bits, zero), jnp.where(low, zero, bits)
    if rem.dtype != f32:
        r0, r1 = pltpu.bitcast(r0, rem.dtype), pltpu.bitcast(r1, rem.dtype)
    return (jnp.concatenate([z[:, 0:MM], r0], axis=1), jnp.concatenate([z[:, MM:2 * MM], r1], axis=1))


def _fold_rem(o):
    o3 = o[:, MM:]
    o3 = o3 + pltpu.roll(o3, 64, 1)
    return jnp.concatenate([o[:, 0:MM], o3[:, 0:DM - MM]], axis=1)


def _seg_softmax(st, mask):
    px, pm = [], []
    for h in range(H):
        sx = st[SEG * h:SEG * (h + 1), :]
        if mask is not None:
            sx = jnp.where(mask, sx, NEG)
        sm = st[H * SEG + NM * h:H * SEG + NM * (h + 1), :]
        s = jnp.concatenate([sx, sm], axis=0)
        e = jnp.exp2(s - jnp.max(s, axis=0, keepdims=True))
        p = e * (1.0 / jnp.sum(e, axis=0, keepdims=True))
        px.append(p[0:SEG])
        pm.append(p[SEG:])
    return jnp.concatenate(px + pm, axis=0)


def _chunk_transpose(t):
    lane = jax.lax.broadcasted_iota(i32, t[0].shape, 1)
    low = lane < 64
    even = (lane & 32) == 0
    u0 = jnp.where(low, t[0], pltpu.roll(t[2], 64, 1))
    u2 = jnp.where(low, pltpu.roll(t[0], 64, 1), t[2])
    u1 = jnp.where(low, t[1], pltpu.roll(t[3], 64, 1))
    u3 = jnp.where(low, pltpu.roll(t[1], 64, 1), t[3])
    return [jnp.where(even, u0, pltpu.roll(u1, 32, 1)), jnp.where(even, pltpu.roll(u0, 96, 1), u1),
            jnp.where(even, u2, pltpu.roll(u3, 32, 1)), jnp.where(even, pltpu.roll(u2, 96, 1), u3)]


def _absorb(wq_hbm, wk_hbm, wv_hbm, wot_hbm, xt_copy, a3, b3, wq_b, wk_b, wv_b, wo_b, sems):
    qscale = (D ** -0.5) * LOG2E
    w32 = [r.bitcast(u32) for r in (wq_hbm, wk_hbm, wv_hbm)]

    def copies(p):
        cs = [pltpu.make_async_copy(w32[j].at[:, p, :], b.at[p], sems.at[j, p])
              for j, b in enumerate((wq_b, wk_b, wv_b))]
        return cs + [pltpu.make_async_copy(wot_hbm.at[pl.ds(2 * p, 2)], wo_b.at[p], sems.at[3, p])]

    for c in copies(0):
        c.start()

    def pre(h, carry):
        p, u = h // 2, h % 2

        @pl.when(u == 0)
        def _():
            for c in copies(p):
                c.wait()

            @pl.when(p == 0)
            def _():
                for c in copies(1):
                    c.start()

            @pl.when(p + 2 < NP)
            def _():
                for c in copies(p + 2):
                    c.start()

            @pl.when(p + 2 == NP)
            def _():
                xt_copy.start()

        q, k, v = (_half(b[p], u) for b in (wq_b, wk_b, wv_b))
        for dst, w in ((a3, _dot_nt(q, k) * qscale), (b3, _dot_nt(wo_b[p, u], v))):
            w = w.astype(bf16)
            dst[p, pl.ds(pl.multiple_of(u * MM, MM), MM), :] = w[0:MM]
            dst[p, pl.ds(pl.multiple_of(2 * MM + 64 * u, 64), 64), :] = w[MM:]
        return carry

    jax.lax.fori_loop(0, H, pre, 0)
    xt_copy.wait()


def _project_tokens(xt, xs, a3, b3, kt, v3):
    per = NKI // (H // 4)
    nb = S // 128 // per

    def proj(i, carry):
        g, t0 = i // per, (i % per) * nb
        rows = pl.ds(pl.multiple_of(t0 * 128, nb * 128), nb * 128)
        xs[rows, :] = xt[:, rows].T
        starts = [(pp, u * MM + c if c < MM else 2 * MM + 64 * u)
                  for c in range(0, DM, 64) for pp in range(2) for u in range(2)]
        for tb in range(nb):
            xb = xt[:, pl.ds(pl.multiple_of((t0 + tb) * 128, 128), 128)]
            lhs = jnp.concatenate([a3[2 * g + pp, r0:r0 + 64, :] for pp, r0 in starts], axis=0)
            z = pltpu.bitcast(_dot(lhs, xb).astype(bf16), u32)
            for c in range(DM // 64):
                t = [z[32 * (4 * c + a):32 * (4 * c + a + 1)] for a in range(4)]
                for b, o in enumerate(_chunk_transpose(t)):
                    kt[g, 4 * (t0 + tb) + b, 64 * c:64 * (c + 1), :] = pltpu.bitcast(o, bf16)
        for pp in range(2):
            v3[2 * g + pp, rows, :] = _dot_nt(xs[rows, :], b3[2 * g + pp]).astype(bf16)
        return carry

    jax.lax.fori_loop(0, NKI, proj, 0)


def _branch_a(m0_ref, o_hbm, acc, xs, a3, b3, kt, v3, o_st, vm, mst, osem):
    def block(i, n):
        return pl.ds(i * n if isinstance(i, int) else pl.multiple_of(i * n, n), n)

    def keys(seg):
        return jnp.concatenate([kt[g, seg] for g in range(5)], axis=1)

    def values(seg):
        rows = block(seg, SEG)
        hs = []
        for p in range(NP):
            hs += list(_split_pair(v3[p, rows, :]))
        return jnp.concatenate(hs + [vm[seg]], axis=0)

    m0 = m0_ref[...].astype(f32)
    mst[...] = jnp.zeros_like(mst)
    mst[0, 0:NM, :] = m0

    def out_copy(j):
        return pltpu.make_async_copy(o_st.at[0:CHAINS, block(j, SEG), :], o_hbm.at[:, block(j, SEG), :], osem.at[j])

    def step(carry):
        n, _ = carry
        j = n % T

        @pl.when(n >= T)
        def _():
            out_copy(j).wait()

        m = mst[j]
        mb = m.astype(bf16)
        zk = [_dot_nt(mb, a3[p]) for p in range(NP)]
        o_st[jnp.minimum(n, CHAINS), :, DM:2 * DM] = acc[:, block(j, T * SEG)].astype(bf16).T
        even = (jax.lax.broadcasted_iota(i32, (32, 128), 1) & NM) == 0
        for c in range(CHAINS):
            cr = slice(NM * c, NM * (c + 1))
            z = jnp.concatenate(
                [jnp.concatenate([zz[cr, u * MM:(u + 1) * MM], zz[cr, 2 * MM:]], axis=1)
                 for zz in zk for u in range(2)], axis=0).astype(bf16).T
            kt[4, c * T + j, 0:MM, :] = z[0:MM]
            kt[4, c * T + j, MM:, :] = pltpu.bitcast(
                jnp.where(even, pltpu.bitcast(z[MM:MM + 64], u32), pltpu.bitcast(z[MM + 64:], u32)), bf16)

        def mem_values(p):
            h0, h1 = _split_pair(_dot_nt(mb, b3[p]))
            for c in range(CHAINS):
                vm[c * T + j, 16 * p:16 * (p + 1), :] = jnp.concatenate(
                    [h0[NM * c:NM * (c + 1)], h1[NM * c:NM * (c + 1)]], axis=0).astype(bf16)

        for p in range(ZV0):
            mem_values(p)
        ss = [_dot(jnp.concatenate([xs[block(c * T + j, SEG), :], m[NM * c:NM * (c + 1)].astype(bf16)], axis=0),
                   keys(c * T + j)) for c in range(CHAINS)]
        for p in range(ZV0, NP):
            mem_values(p)
        kk = jax.lax.broadcasted_iota(i32, (SEG, 128), 0)
        tt = jax.lax.broadcasted_iota(i32, (SEG, 128), 1) % SEG
        sm = [t[SEG:] for t in ss] + ([jnp.zeros((128 - R, NK), f32)] if R < 128 else [])
        pm = _seg_softmax(jnp.concatenate(sm, axis=0).T, None).T
        px = [_seg_softmax(jnp.concatenate([t[0:SEG] for t in ss[c:c + 4]], axis=0).T, kk <= tt).T
              for c in range(0, CHAINS, 4)]
        os_ = []
        for c in range(CHAINS):
            pc = jnp.concatenate([px[c // 4][SEG * (c % 4):SEG * (c % 4 + 1)], pm[NM * c:NM * (c + 1)]], axis=0)
            o = _fold_rem(_dot(pc.astype(bf16), values(c * T + j)))
            o_st[c, block(j, SEG), 0:DM] = o[0:SEG].astype(bf16)
            os_.append(o[SEG:])
        new = jnp.concatenate(os_, axis=0).astype(bf16).astype(f32)
        wrap = jnp.concatenate([m0, new[0:R - NM]], axis=0) if CHAINS > 1 else m0
        jn = (n + 1) % T
        new = jnp.where(jn == 0, wrap, new)
        diff = pltpu.bitcast(new, i32) != pltpu.bitcast(mst[jn], i32)
        changed = jnp.max(diff.astype(i32))
        mst[jn] = new

        @pl.when(n >= T - 1)
        def _():
            def send(jj, carry):
                out_copy(jj).start()
                return carry

            jax.lax.fori_loop(jnp.where(n == T - 1, 0, j), j + 1, send, 0)

        return n + 1, changed

    jax.lax.while_loop(
        lambda c: jnp.logical_and(c[0] < NSEG + T, jnp.logical_or(c[0] < T, c[1] > 0)),
        step, (jnp.int32(0), jnp.int32(1)))


    def drain(j, carry):
        out_copy(j).wait()
        return carry

    jax.lax.fori_loop(0, T, drain, 0)


def _kernel(axt_hbm, m0_ref, awq_hbm, awk_hbm, awv_hbm, awot_hbm,
            bxt_hbm, bc_hbm, bwq_hbm, bwk_hbm, bwv_hbm, bwot_hbm, o_hbm,
            axt, axs, a3, b3, kt, v3, acc, xsem):
    pl.run_scoped(
        functools.partial(_absorb, awq_hbm, awk_hbm, awv_hbm, awot_hbm,
                          pltpu.make_async_copy(axt_hbm, axt, xsem.at[0]), a3, b3),
        pltpu.VMEM((NP, DM, D), u32), pltpu.VMEM((NP, DM, D), u32), pltpu.VMEM((NP, DM, D), u32),
        pltpu.VMEM((NP, 2, DM, D), bf16), pltpu.SemaphoreType.DMA((4, NP)))
    pl.run_scoped(
        functools.partial(_branch_b, bxt_hbm, bc_hbm, bwq_hbm, bwk_hbm, bwv_hbm, bwot_hbm, acc,
                          functools.partial(_project_tokens, axt, axs, a3, b3, kt, v3)),
        pltpu.VMEM((DM, S), bf16), pltpu.VMEM((S, DM), bf16), pltpu.VMEM((S, DC), bf16),
        pltpu.VMEM((2, DM, D), u32), pltpu.VMEM((2, DC, D), u32), pltpu.VMEM((2, DC, D), u32),
        pltpu.VMEM((2, 2, DM, D), bf16), pltpu.VMEM((2, DM, D), bf16), pltpu.VMEM((2, DC, 2 * D), bf16),
        pltpu.VMEM((S, D), bf16), pltpu.VMEM((S, D), bf16), pltpu.VMEM((S, D), bf16),
        pltpu.SemaphoreType.DMA((5, 2)))
    pl.run_scoped(
        functools.partial(_branch_a, m0_ref, o_hbm, acc, axs, a3, b3, kt, v3),
        pltpu.VMEM((CHAINS + 1, T * SEG, 2 * DM), bf16),
        pltpu.VMEM((NSEG, 128, 512), bf16), pltpu.VMEM((T, R, DM), f32),
        pltpu.SemaphoreType.DMA((T,)))


@jax.jit
def pallas_concat_heads__memory_aug_recurrent_mem_tr__compressed_kv_cla__prompt_kernel(
    A_x, A_mem0, A_Wq, A_Wk, A_Wv, A_Wo, A_seg_len, B_x, B_c_kv, B_w_q, B_w_uk, B_w_uv, B_w_o,
):
    del A_seg_len
    assert A_x.shape == (1, S, DM) and B_c_kv.shape == (1, S, DC) and A_Wq.shape == (DM, H, D)
    in_hbm = pl.BlockSpec(memory_space=pltpu.HBM)
    out = pl.pallas_call(
        _kernel,
        out_shape=pltpu.HBM((CHAINS, T * SEG, 2 * DM), bf16),
        in_specs=[in_hbm, pl.BlockSpec(memory_space=pltpu.VMEM)] + [in_hbm] * 10,
        out_specs=in_hbm,
        scratch_shapes=[
            pltpu.VMEM((DM, S), bf16), pltpu.VMEM((S, DM), bf16), pltpu.VMEM((NP, PW, DM), bf16), pltpu.VMEM((NP, PW, DM), bf16),
            pltpu.VMEM((5, NSEG, DM, 128), bf16), pltpu.VMEM((NP, S, PW), bf16),
            pltpu.VMEM((DM, S), f32), pltpu.SemaphoreType.DMA((1,))],
        compiler_params=pltpu.CompilerParams(vmem_limit_bytes=120 * 1024 * 1024),
        name="fused_rmt_mla",
    )(A_x[0].T, A_mem0[0], A_Wq, A_Wk, A_Wv, A_Wo.transpose(0, 2, 1),
      B_x[0].T, B_c_kv[0], B_w_q, B_w_uk, B_w_uv, B_w_o.transpose(0, 2, 1))
    return out.reshape(1, S, 2 * DM)
```
